```python
import jax
import jax.numpy as jnp

def _softmax(x, axis=-1):
    return jax.nn.softmax(x, axis=axis)

def _gelu(x):
    return jax.nn.gelu(x, approximate=True)

def _silu(x):
    return jax.nn.silu(x)

def _sigmoid(x):
    return jax.nn.sigmoid(x)

def _layernorm(x, axis=-1, eps=1e-05):
    m = jnp.mean(x, axis=axis, keepdims=True)
    v = jnp.var(x, axis=axis, keepdims=True)
    return (x - m) / jnp.sqrt(v + eps)

def _scatter_add(tgt, idx, src, axis=0):
    return tgt.at[idx].add(src)

def _segment_sum(src, seg, n):
    return jax.ops.segment_sum(src, seg, n)

class _Rng:

    def __init__(self, key):
        self._k = key

    def _next(self):
        self._k, sub = jax.random.split(self._k)
        return sub

    def normal(self, shape):
        return jax.random.normal(self._next(), shape, dtype=jnp.bfloat16)

    def randint(self, lo, hi, shape):
        return jax.random.randint(self._next(), shape, lo, hi, dtype=jnp.int32)

    def uniform(self, shape, lo=0.0, hi=1.0):
        return jax.random.uniform(self._next(), shape, jnp.bfloat16, lo, hi)

    def permutation(self, n):
        return jax.random.permutation(self._next(), n)
kernel_name = 'recurrent_scan__memory_aug_recurrent_mem_tr__moe_arch_mod__prompt'

def setup_inputs():
    _rng = _Rng(jax.random.key(int.from_bytes(__import__("os").urandom(4), "little")))
    _w = lambda a: (lambda t: t.astype(jnp.bfloat16) if jnp.issubdtype(t.dtype, jnp.floating) else t)(jnp.asarray(a))

    def _A_setup():
        B, S, Dm = (1, 2048, 640)
        H, Dh = (32, 128)
        M, seg = (8, 32)
        seg = min(seg, S)
        S = S // seg * seg
        return {'x': _w((lambda *s: _rng.normal(s) * 0.05)(B, S, Dm)), 'mem0': _w((lambda *s: _rng.normal(s) * 0.05)(B, M, Dm)), 'Wq': _w((lambda *s: _rng.normal(s) * 0.05)(Dm, H, Dh) * Dm ** (-0.5)), 'Wk': _w((lambda *s: _rng.normal(s) * 0.05)(Dm, H, Dh) * Dm ** (-0.5)), 'Wv': _w((lambda *s: _rng.normal(s) * 0.05)(Dm, H, Dh) * Dm ** (-0.5)), 'Wo': _w((lambda *s: _rng.normal(s) * 0.05)(H, Dh, Dm) * (H * Dh) ** (-0.5)), 'seg_len': seg}
    _A_in = _A_setup()

    def _B_setup():
        B, S, D, F, C = (1, 2048, 640, 1728, 8)
        return {'x': _w((lambda *s: _rng.normal(s) * 0.05)(B, S, D)), 'w_r': _w((lambda *s: _rng.normal(s) * 0.05)(D)), 'w_gate': _w((lambda *s: _rng.normal(s) * 0.05)(D, F)), 'w_up': _w((lambda *s: _rng.normal(s) * 0.05)(D, F)), 'w_down': _w((lambda *s: _rng.normal(s) * 0.05)(F, D))}
    _B_in = _B_setup()
    return {'A_x': _A_in['x'], 'A_mem0': _A_in['mem0'], 'A_Wq': _A_in['Wq'], 'A_Wk': _A_in['Wk'], 'A_Wv': _A_in['Wv'], 'A_Wo': _A_in['Wo'], 'A_seg_len': _A_in['seg_len'], 'B_x': _B_in['x'], 'B_w_r': _B_in['w_r'], 'B_w_gate': _B_in['w_gate'], 'B_w_up': _B_in['w_up'], 'B_w_down': _B_in['w_down']}

def reference(A_x, A_mem0, A_Wq, A_Wk, A_Wv, A_Wo, A_seg_len, B_x, B_w_r, B_w_gate, B_w_up, B_w_down):

    def _A_ref(x, mem0, Wq, Wk, Wv, Wo, seg_len):
        B, S, Dm = x.shape
        H, Dh = (Wq.shape[1], Wq.shape[2])
        M = mem0.shape[1]
        scale = Dh ** (-0.5)
        n_seg = S // seg_len
        L = M + seg_len
        idx = jnp.arange(L)
        mask = (idx[:, None] < M) | (idx[:, None] >= idx[None, :])
        mem = mem0
        outs = []
        for s in range(n_seg):
            xs = x[:, s * seg_len:(s + 1) * seg_len, :].copy()
            h = jnp.concatenate([mem, xs], axis=1)
            q = jnp.einsum('btd,dhe->bhte', h, Wq)
            k = jnp.einsum('btd,dhe->bhte', h, Wk)
            v = jnp.einsum('btd,dhe->bhte', h, Wv)
            scores = jnp.einsum('bhqe,bhke->bhqk', q, k) * scale
            scores = jnp.where(mask[None, None], scores, -1000000000.0)
            p = _softmax(scores, axis=-1)
            o = jnp.einsum('bhqk,bhke->bhqe', p, v)
            o = jnp.einsum('bhte,hed->btd', o, Wo)
            mem = o[:, :M, :].copy()
            outs.append(o[:, M:, :])
        return jnp.concatenate(outs, axis=1)

    def _B_ref(x, w_r, w_gate, w_up, w_down):
        B, S, D = x.shape
        C = 8
        r = x @ w_r
        idx = jnp.argsort(-r, axis=-1)[:, :C]
        idx_e = jnp.repeat(idx.reshape(B, C, 1), D, axis=2)
        x_sel = jnp.take_along_axis(x, idx_e, axis=1)
        g = _silu(x_sel @ w_gate)
        u = x_sel @ w_up
        y = g * u @ w_down
        r_sel = _sigmoid(jnp.take_along_axis(r, idx, axis=1))
        y = y * r_sel.reshape(B, C, 1)
        b_off = (jnp.arange(B) * S).reshape(B, 1)
        flat_idx = (idx + b_off).reshape(B * C)
        zero = (x * 0.0).reshape(B * S, D)
        upd = _scatter_add(zero, flat_idx, y.reshape(B * C, D), axis=0)
        return x + upd.reshape(B, S, D)
    x = A_x
    xn = _layernorm(x, axis=-1)
    s = _A_ref(xn, A_mem0, A_Wq, A_Wk, A_Wv, A_Wo, A_seg_len)
    g = _silu(_B_ref(xn, B_w_r, B_w_gate, B_w_up, B_w_down))
    return x + s * g
```

```python
import functools

import jax
import jax.numpy as jnp
from jax import lax
from jax.experimental import pallas as pl
from jax.experimental.pallas import tpu as pltpu

F32 = jnp.float32
BF16 = jnp.bfloat16
U32 = jnp.uint32
I32 = jnp.int32

TOPK = 8
PRE = 8
LN_EPS = 1e-05


def _bf(x):
    return x.astype(BF16).astype(F32)


def _make_kernel(S, D, H, DH, M, SEG, F, cfg):
    NSEG = S // SEG
    L = M + SEG
    MAIN = SEG - PRE
    NPAIR = H // 2
    LAG_QK, LAG_PV = cfg.get("lag", (2, 2))
    OUT_EVERY = cfg.get("out_every", 4)
    LN_ROWS = 128
    scale = DH ** -0.5
    nt_dims = (((1,), (1,)), ((), ()))

    def kernel(x_hbm, mem0_hbm, wq_hbm, wk_hbm, wv_hbm, wo_hbm, wr_hbm, wg_hbm, wu_hbm, wd_hbm,
               out_hbm,
               mem0_v, wr_v, x_v, xn_v, z_v, xpre_v, stage, wqkv, wo_v, pre_v, o_v, wg_v, wu_v, wd_v, xsel_v, out_v,
               sem_x, sem_s, sem_w, sem_o, sem_b, sem_out):
        cp_x = pltpu.make_async_copy(x_hbm, x_v, sem_x)
        cp_x.start()
        cp_s = [pltpu.make_async_copy(wr_hbm, wr_v, sem_s.at[0]),
                pltpu.make_async_copy(mem0_hbm, mem0_v, sem_s.at[1])]
        for c in cp_s:
            c.start()

        def w_copy(p, j):
            src = (wq_hbm, wk_hbm, wv_hbm)[j].bitcast(U32).at[:, p, :]
            return pltpu.make_async_copy(src, stage.at[p, j], sem_w.at[p * 3 + j])

        AHEAD = cfg.get("ahead", 4)
        FIRST = cfg.get("first", 1)

        def w_start(p):
            for j in range(3):
                w_copy(p, j).start()

        for p in range(FIRST):
            w_start(p)
        cp_b = [pltpu.make_async_copy(s, d, sem_b.at[i])
                for i, (s, d) in enumerate(((wg_hbm, wg_v), (wu_hbm, wu_v), (wd_hbm, wd_v)))]
        cp_o = pltpu.make_async_copy(wo_hbm.bitcast(U32), wo_v, sem_o)

        cp_x.wait()
        for p in range(FIRST, AHEAD):
            w_start(p)

        def ln_body(i, c):
            r0 = pl.multiple_of(i * LN_ROWS, LN_ROWS)
            x = x_v[pl.ds(r0, LN_ROWS), :].astype(F32)
            mean = jnp.sum(x, axis=-1, keepdims=True) * (1.0 / D)
            xc = x - mean
            var = jnp.sum(xc * xc, axis=-1, keepdims=True) * (1.0 / D)
            den = _bf(jnp.sqrt(_bf(_bf(var) + _bf(jnp.float32(LN_EPS)))))
            xn = _bf(_bf(x - _bf(mean)) / den)
            xn_v[pl.ds(r0, LN_ROWS), :] = xn
            z_v[pl.ds(r0, LN_ROWS), :] = xn
            n = LN_ROWS // SEG
            tail = jnp.concatenate([xn[k * SEG + MAIN:(k + 1) * SEG] for k in range(n)], axis=0)
            p0 = pl.multiple_of(i * (n * PRE), n * PRE)
            xpre_v[pl.ds(p0, n * PRE), :] = tail.astype(BF16)
            return c

        lax.fori_loop(0, S // LN_ROWS, ln_body, 0)

        for c in cp_s:
            c.wait()
        wr = jnp.broadcast_to(wr_v[...].astype(F32).reshape(1, D), (8, D))
        sub = lax.broadcasted_iota(I32, (8, 128), 0)
        parts = []
        for g in range(S // 1024):
            acc = jnp.zeros((8, 128), F32)
            for j in range(8):
                t = g * 8 + j
                xt = xn_v[t * 128:(t + 1) * 128, :].astype(BF16)
                r = lax.dot_general(wr, xt, nt_dims, preferred_element_type=F32)
                acc = jnp.where(sub == j, r, acc)
            parts.append(acc)
        r = _bf(jnp.concatenate(parts, axis=0))
        bits = (pltpu.bitcast(r, U32) >> 16).astype(I32)
        key = jnp.where(bits >= 0x8000, 0xFFFF - bits, bits + 0x8000)
        key = jnp.where(r == 0.0, 0x8000, key)
        key = jnp.where(r != r, -1, key).astype(F32)
        pos = (lax.broadcasted_iota(I32, r.shape, 0) * 128
               + lax.broadcasted_iota(I32, r.shape, 1)).astype(F32)
        sel = []
        rsel = jnp.zeros((8, 128), F32)
        for j in range(TOPK):
            best = jnp.max(key)
            where = jnp.min(jnp.where(key == best, pos, float(S)))
            hit = pos == where
            rj = jnp.sum(jnp.where(hit, r, 0.0))
            rsel = jnp.where(sub == j, rj, rsel)
            key = jnp.where(hit, -2.0, key)
            idx = where.astype(I32)
            sel.append(idx)
            xsel_v[j:j + 1, :] = xn_v[pl.ds(idx, 1), :]

        def unpack(p):
            for j in range(3):
                w_copy(p, j).wait()
                a = stage[p, j, pl.ds(0, D // 2, stride=2), :]
                b = stage[p, j, pl.ds(1, D // 2, stride=2), :]
                wqkv[2 * p, :, j * DH:(j + 1) * DH] = (a & 0xFFFF) | (b << 16)
                wqkv[2 * p + 1, :, j * DH:(j + 1) * DH] = (a >> 16) | (b & jnp.uint32(0xFFFF0000))

        def project(p):
            for k in range(2):
                h = 2 * p + k
                w = pltpu.bitcast(wqkv[h], BF16)
                pre_v[h] = jnp.dot(xpre_v[...], w, preferred_element_type=F32)

        unpack(0)

        B_AT = cfg.get("b_at", (3, 5, 7, 9))

        def pre_body(p, c):
            @pl.when(p + AHEAD < NPAIR)
            def _():
                w_start(p + AHEAD)

            for at, cp in zip(B_AT, cp_b + [cp_o]):
                @pl.when(p == at)
                def _():
                    cp.start()

            unpack(p + 1)
            project(p)
            return c

        lax.fori_loop(0, NPAIR - 1, pre_body, 0)
        project(NPAIR - 1)

        for c in cp_b:
            c.wait()
        xs = xsel_v[...]
        gate = lax.dot_general(xs, wg_v[...], nt_dims, preferred_element_type=F32)
        up = lax.dot_general(xs, wu_v[...], nt_dims, preferred_element_type=F32)
        act = gate * jax.nn.sigmoid(gate) * up
        y = jnp.dot(act, wd_v[...], preferred_element_type=F32)
        y = y * jax.nn.sigmoid(rsel[:, 0:1])
        zsel = xs + y
        for j in range(TOPK):
            z_v[pl.ds(sel[j], 1), :] = zsel[j:j + 1, :]

        cp_o.wait()
        row = lax.broadcasted_iota(I32, (L, L), 0)
        col = lax.broadcasted_iota(I32, (L, L), 1)
        mask = (row < M) | (row >= col)

        def out_copy(c):
            r0 = pl.multiple_of(c * (OUT_EVERY * SEG), OUT_EVERY * SEG)
            return pltpu.make_async_copy(out_v.at[pl.ds(r0, OUT_EVERY * SEG), :],
                                         out_hbm.at[pl.ds(r0, OUT_EVERY * SEG), :], sem_out)

        def step(s, mem):
            @pl.when(jnp.logical_and(s % OUT_EVERY == 0, s > 0))
            def _():
                out_copy(s // OUT_EVERY - 1).start()

            r0 = pl.multiple_of(s * SEG, SEG)
            p0 = pl.multiple_of(s * PRE, PRE)
            hh = jnp.concatenate([mem, xn_v[pl.ds(r0, MAIN), :]], axis=0).astype(BF16)
            q, k, v, e, inv = {}, {}, {}, {}, {}
            acc = [None]

            def proj(h):
                w = pltpu.bitcast(wqkv[h], BF16)
                t = jnp.dot(hh, w, preferred_element_type=F32)
                t = jnp.concatenate([t, pre_v[h, pl.ds(p0, PRE), :]], axis=0)
                q[h] = t[:, 0:DH]
                k[h] = t[:, DH:2 * DH].astype(BF16)
                v[h] = t[:, 2 * DH:3 * DH].astype(BF16)

            def scores(h):
                sc = lax.dot_general(q.pop(h), k.pop(h), nt_dims, preferred_element_type=F32)
                sc = jnp.where(mask, sc * scale, -1e9)
                ex = jnp.exp(sc - jnp.max(sc, axis=-1, keepdims=True))
                e[h] = ex
                inv[h] = 1.0 / jnp.sum(ex, axis=-1, keepdims=True)

            def values(h):
                o = jnp.dot(e.pop(h), v.pop(h), preferred_element_type=F32)
                o_v[:, h * DH:(h + 1) * DH] = o * inv.pop(h)

            def outproj(h):
                w = pltpu.bitcast(wo_v[h * (DH // 2):(h + 1) * (DH // 2), :], BF16)
                t = jnp.dot(o_v[:, h * DH:(h + 1) * DH], w, preferred_element_type=F32)
                acc[0] = t if acc[0] is None else acc[0] + t

            done = 0
            t = 0
            while done < H:
                if t < H:
                    proj(t)
                if 0 <= t - LAG_QK < H:
                    scores(t - LAG_QK)
                if 0 <= t - LAG_QK - LAG_PV < H:
                    values(t - LAG_QK - LAG_PV)
                if t >= H:
                    n = 0
                    while done < H and n < 3 and done + LAG_QK + LAG_PV + 1 <= t:
                        outproj(done)
                        done += 1
                        n += 1
                t += 1

            res = acc[0]
            z = z_v[pl.ds(r0, SEG), :]
            g = z * jax.nn.sigmoid(z)
            x = x_v[pl.ds(r0, SEG), :].astype(F32)
            out_v[pl.ds(r0, SEG), :] = (x + res[M:] * g).astype(out_v.dtype)
            return res[:M]

        lax.fori_loop(0, NSEG, step, mem0_v[...].astype(F32))
        out_copy(NSEG // OUT_EVERY - 1).start()
        pltpu.make_async_copy(out_v, out_hbm, sem_out).wait()

    return kernel


def build(cfg):
    @functools.partial(jax.jit, static_argnames=("A_seg_len",))
    def fn(A_x, A_mem0, A_Wq, A_Wk, A_Wv, A_Wo, A_seg_len, B_x, B_w_r, B_w_gate, B_w_up, B_w_down):
        del B_x
        B, S, D = A_x.shape
        _, H, DH = A_Wq.shape
        M = A_mem0.shape[1]
        F = B_w_gate.shape[1]
        SEG = int(A_seg_len)
        assert B == 1
        NSEG = S // SEG
        any_spec = pl.BlockSpec(memory_space=pl.ANY)
        vmem_spec = pl.BlockSpec(memory_space=pltpu.VMEM)
        out = pl.pallas_call(
            _make_kernel(S, D, H, DH, M, SEG, F, cfg),
            out_shape=jax.ShapeDtypeStruct((S, D), A_x.dtype),
            in_specs=[any_spec] * 10,
            out_specs=any_spec,
            scratch_shapes=[
                pltpu.VMEM((M, D), BF16),
                pltpu.VMEM((D,), BF16),
                pltpu.VMEM((S, D), BF16),
                pltpu.VMEM((S, D), F32),
                pltpu.VMEM((S, D), F32),
                pltpu.VMEM((NSEG * PRE, D), BF16),
                pltpu.VMEM((H // 2, 3, D, DH), U32),
                pltpu.VMEM((H, D // 2, 3 * DH), U32),
                pltpu.VMEM((H * DH // 2, D), U32),
                pltpu.VMEM((H, NSEG * PRE, 3 * DH), F32),
                pltpu.VMEM((M + SEG, H * DH), F32),
                pltpu.VMEM((F, D), BF16),
                pltpu.VMEM((F, D), BF16),
                pltpu.VMEM((F, D), BF16),
                pltpu.VMEM((TOPK, D), F32),
                pltpu.VMEM((S, D), A_x.dtype),
                pltpu.SemaphoreType.DMA,
                pltpu.SemaphoreType.DMA((2,)),
                pltpu.SemaphoreType.DMA((3 * H // 2,)),
                pltpu.SemaphoreType.DMA,
                pltpu.SemaphoreType.DMA((3,)),
                pltpu.SemaphoreType.DMA,
            ],
            compiler_params=pltpu.CompilerParams(vmem_limit_bytes=120 * 2**20),
        )(A_x.reshape(S, D), A_mem0.reshape(M, D), A_Wq, A_Wk, A_Wv, A_Wo.reshape(H * DH, D),
          B_w_r, B_w_gate.T, B_w_up.T, B_w_down)
        return out.reshape(B, S, D)

    return fn


pallas_recurrent_scan__memory_aug_recurrent_mem_tr__moe_arch_mod__prompt_kernel = build({})
```

```python
import functools

import jax
import jax.numpy as jnp
from jax import lax
from jax.experimental import pallas as pl
from jax.experimental.pallas import tpu as pltpu

F32 = jnp.float32
BF16 = jnp.bfloat16
U32 = jnp.uint32
I32 = jnp.int32

TOPK = 8
PRE = 8
GROUP = 4
LN_EPS = 1e-05


def _bf(x):
    return x.astype(BF16).astype(F32)


def _layernorm(x):
    d = x.shape[-1]
    mean = jnp.sum(x, axis=-1, keepdims=True) * (1.0 / d)
    xc = x - mean
    var = jnp.sum(xc * xc, axis=-1, keepdims=True) * (1.0 / d)
    den = _bf(jnp.sqrt(_bf(_bf(var) + _bf(jnp.float32(LN_EPS)))))
    return _bf(_bf(x - _bf(mean)) / den)


def _make_kernel(S, D, H, DH, M, SEG, F, cfg):
    NSEG = S // SEG
    L = M + SEG
    MAIN = SEG - PRE
    NPAIR = H // 2
    NGROUP = NSEG // GROUP
    NFULL = NPAIR - GROUP // 2
    LAG_QK, LAG_PV = cfg.get("lag", (2, 2))
    EARLY = cfg.get("early", 1)
    RATE = cfg.get("rate", 4)
    LN_ITERS = 8
    TOPK_ITERS = 4
    LN_ROWS = S // LN_ITERS
    AHEAD = cfg.get("ahead", 3)
    XN0 = (NSEG + GROUP) * PRE // 2
    scale = DH ** -0.5
    nt_dims = (((1,), (1,)), ((), ()))
    assert NFULL == 1 + LN_ITERS + 1 + TOPK_ITERS

    def kernel(x_hbm, x4_hbm, mem0_hbm, wq_hbm, wk_hbm, wv_hbm, wo_hbm, wr_hbm, wg_hbm, wu_hbm, wd_hbm,
               out_hbm,
               mem0_v, wr_v, xtail_v, x_v, xx_v, z_v, stage, wqkv, wo_v, pre_v, o_v, g_v,
               wg_v, wu_v, wd_v, xsel_v, out_v, sel_s,
               sem_x, sem_s, sem_w, sem_o, sem_b, sem_out):
        import contextlib
        _scopes = contextlib.ExitStack()
        def mark(name):
            if cfg.get("scopes"):
                _scopes.close()
                if name:
                    _scopes.enter_context(jax.named_scope(name))
        mark("a_start")
        cp_tail = pltpu.make_async_copy(x4_hbm.at[:, SEG // PRE - 1], xtail_v, sem_s.at[2])
        cp_tail.start()

        def w_copy(p, j):
            src = (wq_hbm, wk_hbm, wv_hbm)[j].bitcast(U32).at[:, p, :]
            return pltpu.make_async_copy(src, stage.at[p, j], sem_w.at[p * 3 + j])

        def w_start(p):
            for j in range(3):
                w_copy(p, j).start()

        def x_copy(i):
            r0 = pl.multiple_of(i * LN_ROWS, LN_ROWS)
            return pltpu.make_async_copy(x_hbm.at[pl.ds(r0, LN_ROWS), :], x_v.at[pl.ds(r0, LN_ROWS), :],
                                         sem_x.at[i])

        cp_s = [pltpu.make_async_copy(wr_hbm, wr_v, sem_s.at[0]),
                pltpu.make_async_copy(mem0_hbm, mem0_v, sem_s.at[1])]

        def pieces(src, dst, n, sem):
            rows = dst.shape[0] // n
            return [pltpu.make_async_copy(src.at[pl.ds(i * rows, rows), :], dst.at[pl.ds(i * rows, rows), :],
                                          sem.at[i]) for i in range(n)]

        late = (pieces(wg_hbm, wg_v, 2, sem_b.at[pl.ds(0, 2)]) + pieces(wu_hbm, wu_v, 2, sem_b.at[pl.ds(2, 2)])
                + pieces(wd_hbm, wd_v, 2, sem_b.at[pl.ds(4, 2)]) + pieces(wo_hbm.bitcast(U32), wo_v, 4, sem_o))

        def xn_rows(r0, n):
            return pltpu.bitcast(xx_v[pl.ds(XN0 + r0, n), :], F32)

        def w_wait(p):
            for j in range(3):
                w_copy(p, j).wait()

        def unpack(p, j):
            a = stage[p, j, pl.ds(0, D // 2, stride=2), :]
            b = stage[p, j, pl.ds(1, D // 2, stride=2), :]
            wqkv[2 * p, :, j * DH:(j + 1) * DH] = (a & 0xFFFF) | (b << 16)
            wqkv[2 * p + 1, :, j * DH:(j + 1) * DH] = (a >> 16) | (b & jnp.uint32(0xFFFF0000))

        def project(h, r0, rows):
            lhs = pltpu.bitcast(xx_v[pl.ds(r0 // 2, rows // 2), :], BF16)
            w = pltpu.bitcast(wqkv[h], BF16)
            pre_v[h, pl.ds(r0, rows), :] = jnp.dot(lhs, w, preferred_element_type=F32)

        NCHUNK = cfg.get("nchunk", 8)
        CHUNK = NSEG * PRE // NCHUNK

        def project_pair(p, jobs):
            n = 2 * NCHUNK
            m = n - cfg.get("free", 2)
            for c in range(n):
                project(2 * p + c // NCHUNK, (c % NCHUNK) * CHUNK, CHUNK)
                if c < m:
                    for job in jobs[c * len(jobs) // m:(c + 1) * len(jobs) // m]:
                        job()

        def unpack_jobs(p):
            return [functools.partial(unpack, p, j) for j in range(3)]

        mark('b_wait_tail')
        cp_tail.wait()
        mark('c_tail_ln')
        w_start(0)

        def tail_body(i, c):
            n = 16
            xt = xtail_v[pl.ds(i * n, n)].astype(F32).reshape(n * PRE, D)
            r0 = pl.multiple_of(i * (n * PRE // 2), n * PRE // 2)
            xx_v[pl.ds(r0, n * PRE // 2), :] = pltpu.bitcast(_layernorm(xt).astype(BF16), U32)
            return c

        lax.fori_loop(0, NSEG // 16, tail_body, 0)
        xx_v[NSEG * PRE // 2:XN0, :] = jnp.zeros((GROUP * PRE // 2, D), U32)
        mark('d_unpack0')
        w_start(1)
        x_copy(0).start()
        w_wait(0)
        for job in unpack_jobs(0):
            job()
        mark('e_p0')

        project(0, 0, NSEG * PRE)
        w_wait(1)
        w_start(2)
        x_copy(1).start()
        for c in cp_s:
            c.start()
        w_start(3)
        for c in range(4):
            project(1, c * (NSEG * PRE // 4), NSEG * PRE // 4)
            if c < 3:
                unpack(1, c)
        mark('g_ln_loop')
        LN_PIECES = cfg.get("ln_pieces", 8)

        def ln_body(i, c):
            p = i + 1
            w_wait(p + 1)

            x_copy(i).wait()

            @pl.when(i + 2 < LN_ITERS)
            def _():
                x_copy(i + 2).start()

            w_start(i + 4)
            for at, cp in enumerate(late[:6]):
                @pl.when(i == at + 2)
                def _():
                    cp.start()

            def ln(t):
                n = LN_ROWS // LN_PIECES
                r0 = pl.multiple_of(i * LN_ROWS + t * n, n)
                xn = _layernorm(x_v[pl.ds(r0, n), :].astype(F32))
                xx_v[pl.ds(XN0 + r0, n), :] = pltpu.bitcast(xn, U32)
                z_v[pl.ds(r0, n), :] = xn

            project_pair(p, unpack_jobs(p + 1) + [functools.partial(ln, t) for t in range(LN_PIECES)])
            return c

        lax.fori_loop(0, LN_ITERS, ln_body, 0)

        mark('h_router')
        p_r = 1 + LN_ITERS
        w_wait(p_r + 1)
        for c in cp_s:
            c.wait()
        w_start(LN_ITERS + 4)
        late[6].start()
        sub = lax.broadcasted_iota(I32, (8, 128), 0)
        wr = jnp.broadcast_to(wr_v[...].astype(F32).reshape(1, D), (8, D))
        parts = []
        for g in range(S // 1024):
            acc = jnp.zeros((8, 128), F32)
            for j in range(8):
                t = g * 8 + j
                xt = xn_rows(t * 128, 128).astype(BF16)
                r = lax.dot_general(wr, xt, nt_dims, preferred_element_type=F32)
                acc = jnp.where(sub == j, r, acc)
            parts.append(acc)
        r = _bf(jnp.concatenate(parts, axis=0))
        bits = (pltpu.bitcast(r, U32) >> 16).astype(I32)
        key = jnp.where(bits >= 0x8000, 0xFFFF - bits, bits + 0x8000)
        key = jnp.where(r == 0.0, 0x8000, key)
        key = jnp.where(r != r, -1, key).astype(F32)
        pos = (lax.broadcasted_iota(I32, r.shape, 0) * 128
               + lax.broadcasted_iota(I32, r.shape, 1)).astype(F32)
        project_pair(p_r, unpack_jobs(p_r + 1))

        mark('i_topk_loop')
        PICKS = TOPK // TOPK_ITERS

        def all_reduce(op, t):
            return op(op(t, axis=1, keepdims=True), axis=0, keepdims=True)

        def topk_body(i, carry):
            st = {"key": carry[0], "rsel": carry[1]}
            p = p_r + 1 + i
            w_wait(p + 1)
            for at, cp in enumerate(late[7:]):
                @pl.when(i == at)
                def _():
                    w_start(LN_ITERS + 5 + at)
                    cp.start()

            def best():
                st["best"] = all_reduce(jnp.max, st["key"])

            def first():
                st["where"] = all_reduce(jnp.min, jnp.where(st["key"] == st["best"], pos, float(S)))

            def take(j):
                hit = pos == st["where"]
                st["rsel"] = jnp.where(sub == j, all_reduce(jnp.sum, jnp.where(hit, r, 0.0)), st["rsel"])
                st["key"] = jnp.where(hit, -2.0, st["key"])
                idx = jnp.clip(st["where"].astype(I32)[0, 0], 0, S - 1)
                sel_s[j] = idx
                xsel_v[pl.ds(j, 1), :] = xn_rows(idx, 1)

            jobs = []
            for t in range(PICKS):
                jobs += [best, first, functools.partial(take, i * PICKS + t)]
            u = unpack_jobs(p + 1)
            jobs = jobs[:3] + [u[0]] + jobs[3:] + u[1:]
            project_pair(p, jobs)
            return st["key"], st["rsel"]

        _, rsel = lax.fori_loop(0, TOPK_ITERS, topk_body, (key, jnp.zeros((8, 128), F32)))
        mark('j_rest')
        for p in range(NFULL + 1, NPAIR):
            w_wait(p)
            for job in unpack_jobs(p):
                job()
        for h in range(2 * NFULL, H):
            project(h, 0, GROUP * PRE)

        mark('k_wait_b')
        for c in late[:6]:
            c.wait()
        mark('l_mlp')
        xs = xsel_v[...]
        gate = lax.dot_general(xs, wg_v[...], nt_dims, preferred_element_type=F32)
        up = lax.dot_general(xs, wu_v[...], nt_dims, preferred_element_type=F32)
        act = gate * jax.nn.sigmoid(gate) * up
        y = jnp.dot(act, wd_v[...], preferred_element_type=F32)
        y = y * jax.nn.sigmoid(rsel[:, 0:1])
        zsel = xs + y
        for j in range(TOPK):
            z_v[pl.ds(sel_s[j], 1), :] = zsel[j:j + 1, :]

        mark('m_wait_wo')
        for c in late[6:]:
            c.wait()
        mark('n_scan')
        row = lax.broadcasted_iota(I32, (L, L), 0)
        col = lax.broadcasted_iota(I32, (L, L), 1)
        mask = (row < M) | (row >= col)

        def out_copy(c):
            r0 = pl.multiple_of(c * (GROUP * SEG), GROUP * SEG)
            return pltpu.make_async_copy(out_v.at[pl.ds(r0, GROUP * SEG), :],
                                         out_hbm.at[pl.ds(r0, GROUP * SEG), :], sem_out)

        def step(grp, sub_step, mem):
            s = grp * GROUP + sub_step
            r0 = pl.multiple_of(s * SEG, SEG)
            p0 = pl.multiple_of(s * PRE, PRE)
            hh = jnp.concatenate([mem, xn_rows(r0, MAIN)], axis=0).astype(BF16)
            q, k, v, e, inv = {}, {}, {}, {}, {}
            acc = [None]

            def proj(h):
                if cfg.get("split3"):
                    t = jnp.concatenate([
                        jnp.dot(hh, pltpu.bitcast(wqkv[h, :, j * DH:(j + 1) * DH], BF16), preferred_element_type=F32)
                        for j in range(3)], axis=1)
                else:
                    t = jnp.dot(hh, pltpu.bitcast(wqkv[h], BF16), preferred_element_type=F32)
                t = jnp.concatenate([t, pre_v[h, pl.ds(p0, PRE), :]], axis=0)
                q[h] = t[:, 0:DH]
                k[h] = t[:, DH:2 * DH].astype(BF16)
                v[h] = t[:, 2 * DH:3 * DH].astype(BF16)

            def scores(h):
                sc = lax.dot_general(q.pop(h), k.pop(h), nt_dims, preferred_element_type=F32)
                sc = jnp.where(mask, sc * scale, -1e9)
                ex = jnp.exp(sc - jnp.max(sc, axis=-1, keepdims=True))
                e[h] = ex
                inv[h] = 1.0 / jnp.sum(ex, axis=-1, keepdims=True)

            def values(h):
                o = jnp.dot(e.pop(h), v.pop(h), preferred_element_type=F32)
                o_v[:, h * DH:(h + 1) * DH] = o * inv.pop(h)

            def outproj(h, n):
                w = pltpu.bitcast(wo_v[h * (DH // 2):(h + n) * (DH // 2), :], BF16)
                t = jnp.dot(o_v[:, h * DH:(h + n) * DH], w, preferred_element_type=F32)
                acc[0] = t if acc[0] is None else acc[0] + t

            done = 0
            t = 0
            GO = cfg.get("go", 1)
            while done < H:
                for what in cfg.get("order", "psvo"):
                    if what == "p" and t < H:
                        proj(t)
                    if what == "s" and 0 <= t - LAG_QK < H:
                        scores(t - LAG_QK)
                    if what == "v" and 0 <= t - LAG_QK - LAG_PV < H:
                        values(t - LAG_QK - LAG_PV)
                    if what == "o" and t >= H - EARLY:
                        n = 0
                        while done < H and n < RATE and done + GO - 1 + LAG_QK + LAG_PV + 1 <= t:
                            outproj(done, GO)
                            done += GO
                            n += GO
                if t == cfg.get("g_at", 8):
                    z = z_v[pl.ds(r0, SEG), :]
                    g_v[...] = z * jax.nn.sigmoid(z)
                t += 1

            hf = H - GROUP + sub_step
            f0 = pl.multiple_of((grp + 1) * (GROUP * PRE), GROUP * PRE)
            f1 = pl.multiple_of((grp + 1) * (GROUP * PRE // 2), GROUP * PRE // 2)
            pre_v[hf, pl.ds(f0, GROUP * PRE), :] = jnp.dot(
                pltpu.bitcast(xx_v[pl.ds(f1, GROUP * PRE // 2), :], BF16),
                pltpu.bitcast(wqkv[hf], BF16), preferred_element_type=F32)

            res = acc[0]
            x = x_v[pl.ds(r0, SEG), :].astype(F32)
            out_v[pl.ds(r0, SEG), :] = (x + res[M:] * g_v[...]).astype(out_v.dtype)
            return res[:M]

        UNROLL = cfg.get("unroll", GROUP)

        def group_body(grp, mem):
            if UNROLL == GROUP:
                for k in range(GROUP):
                    mem = step(grp, k, mem)
            else:
                def inner(i, mem):
                    for k in range(UNROLL):
                        mem = step(grp, i * UNROLL + k, mem)
                    return mem
                mem = lax.fori_loop(0, GROUP // UNROLL, inner, mem)
            out_copy(grp).start()
            return mem

        ngroup = cfg.get("steps", NGROUP)
        lax.fori_loop(0, ngroup, group_body, mem0_v[...].astype(F32))
        mark('o_out')
        if ngroup == NGROUP:
            pltpu.make_async_copy(out_v, out_hbm, sem_out).wait()
        else:
            for c in range(ngroup):
                out_copy(c).wait()
        mark(None)

    return kernel


def build(cfg):
    @functools.partial(jax.jit, static_argnames=("A_seg_len",))
    def fn(A_x, A_mem0, A_Wq, A_Wk, A_Wv, A_Wo, A_seg_len, B_x, B_w_r, B_w_gate, B_w_up, B_w_down):
        del B_x
        B, S, D = A_x.shape
        _, H, DH = A_Wq.shape
        M = A_mem0.shape[1]
        F = B_w_gate.shape[1]
        SEG = int(A_seg_len)
        assert B == 1
        NSEG = S // SEG
        any_spec = pl.BlockSpec(memory_space=pl.ANY)
        out = pl.pallas_call(
            _make_kernel(S, D, H, DH, M, SEG, F, cfg),
            out_shape=jax.ShapeDtypeStruct((S, D), A_x.dtype),
            in_specs=[any_spec] * 11,
            out_specs=any_spec,
            scratch_shapes=[
                pltpu.VMEM((M, D), BF16),
                pltpu.VMEM((D,), BF16),
                pltpu.VMEM((NSEG, PRE, D), BF16),
                pltpu.VMEM((S, D), BF16),
                pltpu.VMEM(((NSEG + GROUP) * PRE // 2 + S, D), U32),
                pltpu.VMEM((S, D), F32),
                pltpu.VMEM((H // 2, 3, D, DH), U32),
                pltpu.VMEM((H, D // 2, 3 * DH), U32),
                pltpu.VMEM((H * DH // 2, D), U32),
                pltpu.VMEM((H, (NSEG + GROUP) * PRE, 3 * DH), F32),
                pltpu.VMEM((M + SEG, H * DH), F32),
                pltpu.VMEM((SEG, D), F32),
                pltpu.VMEM((F, D), BF16),
                pltpu.VMEM((F, D), BF16),
                pltpu.VMEM((F, D), BF16),
                pltpu.VMEM((TOPK, D), F32),
                pltpu.VMEM((S, D), A_x.dtype),
                pltpu.SMEM((TOPK,), I32),
                pltpu.SemaphoreType.DMA((8,)),
                pltpu.SemaphoreType.DMA((3,)),
                pltpu.SemaphoreType.DMA((3 * H // 2,)),
                pltpu.SemaphoreType.DMA((4,)),
                pltpu.SemaphoreType.DMA((6,)),
                pltpu.SemaphoreType.DMA,
            ],
            compiler_params=pltpu.CompilerParams(
                vmem_limit_bytes=120 * 2**20,
                disable_bounds_checks=cfg.get("nobc", False), flags=cfg.get("flags")),
        )(A_x.reshape(S, D), A_x.reshape(NSEG, SEG // PRE, PRE, D), A_mem0.reshape(M, D),
          A_Wq, A_Wk, A_Wv, A_Wo.reshape(H * DH, D),
          B_w_r, B_w_gate.T, B_w_up.T, B_w_down)
        return out.reshape(B, S, D)

    return fn


pallas_recurrent_scan__memory_aug_recurrent_mem_tr__moe_arch_mod__prompt_kernel = build({})
```

```python
import functools

import jax
import jax.numpy as jnp
from jax import lax
from jax.experimental import pallas as pl
from jax.experimental.pallas import tpu as pltpu

F32 = jnp.float32
BF16 = jnp.bfloat16
U32 = jnp.uint32
I32 = jnp.int32

TOPK = 8
PRE = 8
GROUP = 4
LN_EPS = 1e-05


def _bf(x):
    return x.astype(BF16).astype(F32)


def _layernorm(x):
    d = x.shape[-1]
    mean = jnp.sum(x, axis=-1, keepdims=True) * (1.0 / d)
    xc = x - mean
    var = jnp.sum(xc * xc, axis=-1, keepdims=True) * (1.0 / d)
    den = _bf(jnp.sqrt(_bf(_bf(var) + _bf(jnp.float32(LN_EPS)))))
    return _bf(_bf(x - _bf(mean)) / den)


def _make_kernel(S, D, H, DH, M, SEG, F, cfg):
    NSEG = S // SEG
    L = M + SEG
    MAIN = SEG - PRE
    NPAIR = H // 2
    NGROUP = NSEG // GROUP
    NFULL = NPAIR - GROUP // 2
    LAG_QK, LAG_PV = cfg.get("lag", (3, 3))
    EARLY = cfg.get("early", 1)
    RATE = cfg.get("rate", 4)
    LN_ITERS = 8
    TOPK_ITERS = 3
    LN_ROWS = S // LN_ITERS
    AHEAD = cfg.get("ahead", 3)
    XN0 = (NSEG + GROUP) * PRE // 2
    scale = DH ** -0.5
    nt_dims = (((1,), (1,)), ((), ()))
    assert NFULL == 1 + LN_ITERS + 1 + TOPK_ITERS + 1

    def kernel(x_hbm, x4_hbm, mem0_hbm, wq_hbm, wk_hbm, wv_hbm, wo_hbm, wr_hbm, wg_hbm, wu_hbm, wd_hbm,
               out_hbm,
               mem0_v, wr_v, xtail_v, x_v, xx_v, z_v, stage, wqkv, wo_v, pre_v, o_v, g_v,
               wg_v, wu_v, wd_v, xsel_v, out_v, sel_s,
               sem_x, sem_s, sem_w, sem_o, sem_b, sem_out):
        import contextlib
        _scopes = contextlib.ExitStack()
        def mark(name):
            if cfg.get("scopes"):
                _scopes.close()
                if name:
                    _scopes.enter_context(jax.named_scope(name))
        mark("a_start")
        cp_tail = pltpu.make_async_copy(x4_hbm.at[:, SEG // PRE - 1], xtail_v, sem_s.at[2])
        cp_tail.start()

        def w_copy(p, j):
            src = (wq_hbm, wk_hbm, wv_hbm)[j].bitcast(U32).at[:, p, :]
            return pltpu.make_async_copy(src, stage.at[p, j], sem_w.at[p * 3 + j])

        def w_start(p):
            for j in range(3):
                w_copy(p, j).start()

        def x_copy(i):
            r0 = pl.multiple_of(i * LN_ROWS, LN_ROWS)
            return pltpu.make_async_copy(x_hbm.at[pl.ds(r0, LN_ROWS), :], x_v.at[pl.ds(r0, LN_ROWS), :],
                                         sem_x.at[i])

        cp_s = [pltpu.make_async_copy(wr_hbm, wr_v, sem_s.at[0]),
                pltpu.make_async_copy(mem0_hbm, mem0_v, sem_s.at[1])]

        def pieces(src, dst, n, sem):
            rows = dst.shape[0] // n
            return [pltpu.make_async_copy(src.at[pl.ds(i * rows, rows), :], dst.at[pl.ds(i * rows, rows), :],
                                          sem.at[i]) for i in range(n)]

        late = (pieces(wg_hbm, wg_v, 2, sem_b.at[pl.ds(0, 2)]) + pieces(wu_hbm, wu_v, 2, sem_b.at[pl.ds(2, 2)])
                + pieces(wd_hbm, wd_v, 2, sem_b.at[pl.ds(4, 2)]) + pieces(wo_hbm.bitcast(U32), wo_v, 4, sem_o))

        def w_wait(p):
            for j in range(3):
                w_copy(p, j).wait()

        def unpack(p, j):
            a = stage[p, j, pl.ds(0, D // 2, stride=2), :]
            b = stage[p, j, pl.ds(1, D // 2, stride=2), :]
            wqkv[2 * p, :, j * DH:(j + 1) * DH] = (a & 0xFFFF) | (b << 16)
            wqkv[2 * p + 1, :, j * DH:(j + 1) * DH] = (a >> 16) | (b & jnp.uint32(0xFFFF0000))

        def unpack_jobs(p):
            return [functools.partial(unpack, p, j) for j in range(3)]

        def project(h, r0, rows, j=None):
            cols = slice(None) if j is None else slice(j * DH, (j + 1) * DH)
            lhs = pltpu.bitcast(xx_v[pl.ds(r0 // 2, rows // 2), :], BF16)
            w = pltpu.bitcast(wqkv[h, :, cols], BF16)
            pre_v[h, pl.ds(r0, rows), cols] = jnp.dot(lhs, w, preferred_element_type=F32)

        NCHUNK = cfg.get("nchunk", 8)
        CHUNK = NSEG * PRE // NCHUNK

        def project_pair(p, jobs, fine=False, free=2):
            parts = [(c, j) for c in range(2 * NCHUNK) for j in (range(3) if fine else (None,))]
            m = len(parts) - free
            for i, (c, j) in enumerate(parts):
                project(2 * p + c // NCHUNK, (c % NCHUNK) * CHUNK, CHUNK, j)
                if i < m:
                    for job in jobs[i * len(jobs) // m:(i + 1) * len(jobs) // m]:
                        job()

        def ln_tail(i, n):
            xn = _layernorm(xtail_v[i * n:(i + 1) * n].astype(F32).reshape(n * PRE, D))
            xx_v[i * n * PRE // 2:(i + 1) * n * PRE // 2, :] = pltpu.bitcast(xn.astype(BF16), U32)
            for k in range(n):
                z_v[pl.ds((i * n + k) * SEG + MAIN, PRE), :] = xn[k * PRE:(k + 1) * PRE]

        mark('b_wait_tail')
        w_start(0)
        cp_tail.wait()
        w_wait(0)
        mark('e_p0')
        w_start(1)
        x_copy(0).start()
        w_start(2)
        NQ = cfg.get("nq", 4)
        ln_tail(0, NSEG // NQ)
        for job in unpack_jobs(0):
            job()
        for i in range(NQ):
            project(0, i * (NSEG * PRE // NQ), NSEG * PRE // NQ)
            if i + 1 < NQ:
                ln_tail(i + 1, NSEG // NQ)
            project(1, i * (NSEG * PRE // NQ), NSEG * PRE // NQ)
        xx_v[NSEG * PRE // 2:XN0, :] = jnp.zeros((GROUP * PRE // 2, D), U32)
        mark('f_unpack1')
        w_wait(1)
        w_start(3)
        x_copy(1).start()
        for c in cp_s:
            c.start()
        for job in unpack_jobs(1):
            job()

        mark('g_ln_loop')

        def ln_body(i, c):
            p = i + 1
            w_wait(p + 1)
            x_copy(i).wait()

            @pl.when(i + 2 < LN_ITERS)
            def _():
                x_copy(i + 2).start()

            w_start(i + 4)
            for at, cp in enumerate(late[:6]):
                @pl.when(i == at + 2)
                def _():
                    cp.start()

            def ln(t):
                seg = i * (LN_ROWS // SEG) + t
                r0 = pl.multiple_of(seg * SEG, SEG)
                xn = _layernorm(x_v[pl.ds(r0, SEG), :].astype(F32)[:MAIN])
                xx_v[pl.ds(pl.multiple_of(XN0 + seg * MAIN, 8), MAIN), :] = pltpu.bitcast(xn, U32)
                z_v[pl.ds(r0, MAIN), :] = xn

            lns = [functools.partial(ln, t) for t in range(LN_ROWS // SEG)]
            project_pair(p, unpack_jobs(p + 1) + lns, free=cfg.get("free", 2))
            return c

        lax.fori_loop(0, LN_ITERS, ln_body, 0)

        mark('h_router')
        p_r = 1 + LN_ITERS
        w_wait(p_r + 1)
        for c in cp_s:
            c.wait()
        w_start(LN_ITERS + 4)
        late[6].start()
        sub = lax.broadcasted_iota(I32, (8, 128), 0)
        wr = jnp.broadcast_to(wr_v[...].astype(F32).reshape(1, D), (8, D))
        parts = [jnp.zeros((8, 128), F32) for _ in range(S // 1024)]

        def score(t):
            xt = z_v[t * 128:(t + 1) * 128, :].astype(BF16)
            r = lax.dot_general(wr, xt, nt_dims, preferred_element_type=F32)
            parts[t // 8] = jnp.where(sub == t % 8, r, parts[t // 8])

        project_pair(p_r, [functools.partial(score, t) for t in range(S // 128)] + unpack_jobs(p_r + 1),
                     fine=True, free=cfg.get("free_r", 16))
        r = _bf(jnp.concatenate(parts, axis=0))
        bits = (pltpu.bitcast(r, U32) >> 16).astype(I32)
        key = jnp.where(bits >= 0x8000, 0xFFFF - bits, bits + 0x8000)
        key = jnp.where(r == 0.0, 0x8000, key)
        key = jnp.where(r != r, -1, key).astype(F32)
        pos = (lax.broadcasted_iota(I32, r.shape, 0) * 128
               + lax.broadcasted_iota(I32, r.shape, 1)).astype(F32)

        mark('i_topk_loop')
        PICKS = -(-TOPK // TOPK_ITERS)

        def all_reduce(op, t):
            return op(op(t, axis=1, keepdims=True), axis=0, keepdims=True)

        def topk_body(i, carry):
            st = {"key": carry[0], "rsel": carry[1]}
            p = p_r + 1 + i
            w_wait(p + 1)
            w_start(LN_ITERS + 5 + i)
            for at, cp in enumerate(late[7:]):
                @pl.when(i == at)
                def _():
                    cp.start()

            def best():
                st["best"] = all_reduce(jnp.max, st["key"])

            def first():
                st["where"] = all_reduce(jnp.min, jnp.where(st["key"] == st["best"], pos, float(S)))

            def take(j):
                hit = pos == st["where"]
                st["rsel"] = jnp.where(sub == j, all_reduce(jnp.sum, jnp.where(hit, r, 0.0)), st["rsel"])
                st["key"] = jnp.where(hit, -2.0, st["key"])
                idx = jnp.clip(st["where"].astype(I32)[0, 0], 0, S - 1)
                sel_s[j] = idx
                xsel_v[pl.ds(j, 1), :] = z_v[pl.ds(idx, 1), :]

            jobs = []
            u = unpack_jobs(p + 1)
            for t in range(PICKS):
                jobs += [best, first, functools.partial(take, i * PICKS + t)] + u[t:t + 1]
            project_pair(p, jobs, free=cfg.get("free_k", 2))
            return st["key"], st["rsel"]

        _, rsel = lax.fori_loop(0, TOPK_ITERS, topk_body, (key, jnp.zeros((8, 128), F32)))

        mark('k_wait_b')
        for c in late[:6]:
            c.wait()
        for p in range(NFULL, NPAIR):
            w_wait(p)
        mark('l_mlp')
        xs = xsel_v[0:TOPK, :]
        mlp = {}

        def hidden(name, ref, t):
            w = ref[t * 128:min((t + 1) * 128, F), :]
            mlp[name, t] = lax.dot_general(xs, w, nt_dims, preferred_element_type=F32)

        def down(t):
            gate = mlp.pop(("g", t))
            act = gate * jax.nn.sigmoid(gate) * mlp.pop(("u", t))
            y = jnp.dot(act, wd_v[t * 128:min((t + 1) * 128, F), :], preferred_element_type=F32)
            mlp["y"] = y + mlp["y"] if "y" in mlp else y

        jobs = []
        NF = -(-F // 128)
        for t in range(NF + 1):
            if t < NF:
                jobs += [functools.partial(hidden, "g", wg_v, t), functools.partial(hidden, "u", wu_v, t)]
            if t > 0:
                jobs += [functools.partial(down, t - 1)]
        for p in range(NFULL, NPAIR):
            for k, job in enumerate(unpack_jobs(p)):
                jobs.insert(4 * k + 2, job)
        project_pair(NFULL - 1, jobs, fine=True, free=cfg.get("free_m", 0))
        for h in range(2 * NFULL, H):
            project(h, 0, GROUP * PRE)
        zsel = xs + mlp["y"] * jax.nn.sigmoid(rsel[:, 0:1])
        for j in range(TOPK):
            z_v[pl.ds(sel_s[j], 1), :] = zsel[j:j + 1, :]

        mark('m_wait_wo')
        for c in late[6:]:
            c.wait()
        mark('n_scan')
        row = lax.broadcasted_iota(I32, (L, L), 0)
        col = lax.broadcasted_iota(I32, (L, L), 1)
        mask = (row < M) | (row >= col)

        def out_copy(c):
            r0 = pl.multiple_of(c * (GROUP * SEG), GROUP * SEG)
            return pltpu.make_async_copy(out_v.at[pl.ds(r0, GROUP * SEG), :],
                                         out_hbm.at[pl.ds(r0, GROUP * SEG), :], sem_out)

        def step(grp, sub_step, mem):
            s = grp * GROUP + sub_step
            r0 = pl.multiple_of(s * SEG, SEG)
            p0 = pl.multiple_of(s * PRE, PRE)
            xm = pltpu.bitcast(xx_v[pl.ds(pl.multiple_of(XN0 + s * MAIN, 8), MAIN), :], F32)
            hh = jnp.concatenate([mem, xm], axis=0).astype(BF16)
            q, k, v, e, inv = {}, {}, {}, {}, {}
            acc = [None]

            def proj(h):
                if cfg.get("split3"):
                    t = jnp.concatenate([
                        jnp.dot(hh, pltpu.bitcast(wqkv[h, :, j * DH:(j + 1) * DH], BF16), preferred_element_type=F32)
                        for j in range(3)], axis=1)
                else:
                    t = jnp.dot(hh, pltpu.bitcast(wqkv[h], BF16), preferred_element_type=F32)
                t = jnp.concatenate([t, pre_v[h, pl.ds(p0, PRE), :]], axis=0)
                q[h] = t[:, 0:DH]
                k[h] = t[:, DH:2 * DH].astype(BF16)
                v[h] = t[:, 2 * DH:3 * DH].astype(BF16)

            def scores(h):
                sc = lax.dot_general(q.pop(h), k.pop(h), nt_dims, preferred_element_type=F32)
                sc = jnp.where(mask, sc * scale, -1e9)
                ex = jnp.exp(sc - jnp.max(sc, axis=-1, keepdims=True))
                e[h] = ex
                inv[h] = 1.0 / jnp.sum(ex, axis=-1, keepdims=True)

            def values(h):
                o = jnp.dot(e.pop(h), v.pop(h), preferred_element_type=F32)
                o_v[:, h * DH:(h + 1) * DH] = o * inv.pop(h)

            def outproj(h, n):
                w = pltpu.bitcast(wo_v[h * (DH // 2):(h + n) * (DH // 2), :], BF16)
                t = jnp.dot(o_v[:, h * DH:(h + n) * DH], w, preferred_element_type=F32)
                acc[0] = t if acc[0] is None else acc[0] + t

            done = 0
            t = 0
            GO = cfg.get("go", 2)
            while done < H:
                for what in cfg.get("order", "psvo"):
                    if what == "p" and t < H:
                        proj(t)
                    if what == "s" and 0 <= t - LAG_QK < H:
                        scores(t - LAG_QK)
                    if what == "v" and 0 <= t - LAG_QK - LAG_PV < H:
                        values(t - LAG_QK - LAG_PV)
                    if what == "o" and t >= H - EARLY:
                        n = 0
                        while done < H and n < RATE and done + GO - 1 + LAG_QK + LAG_PV + 1 <= t:
                            outproj(done, GO)
                            done += GO
                            n += GO
                if t == cfg.get("g_at", 8):
                    z = z_v[pl.ds(r0, SEG), :]
                    g_v[...] = z * jax.nn.sigmoid(z)
                t += 1

            hf = H - GROUP + sub_step
            f0 = pl.multiple_of((grp + 1) * (GROUP * PRE), GROUP * PRE)
            f1 = pl.multiple_of((grp + 1) * (GROUP * PRE // 2), GROUP * PRE // 2)
            pre_v[hf, pl.ds(f0, GROUP * PRE), :] = jnp.dot(
                pltpu.bitcast(xx_v[pl.ds(f1, GROUP * PRE // 2), :], BF16),
                pltpu.bitcast(wqkv[hf], BF16), preferred_element_type=F32)

            res = acc[0]
            x = x_v[pl.ds(r0, SEG), :].astype(F32)
            out_v[pl.ds(r0, SEG), :] = (x + res[M:] * g_v[...]).astype(out_v.dtype)
            return res[:M]

        UG = cfg.get("ug", 1)

        def group_body(i, mem):
            for g in range(UG):
                for k in range(GROUP):
                    mem = step(i * UG + g, k, mem)
            for g in range(UG):
                out_copy(i * UG + g).start()
            return mem

        ngroup = cfg.get("steps", NGROUP)
        lax.fori_loop(0, ngroup // UG, group_body, mem0_v[...].astype(F32))
        mark('o_out')
        if ngroup == NGROUP:
            pltpu.make_async_copy(out_v, out_hbm, sem_out).wait()
        else:
            for c in range(ngroup):
                out_copy(c).wait()
        mark(None)

    return kernel


def build(cfg):
    @functools.partial(jax.jit, static_argnames=("A_seg_len",))
    def fn(A_x, A_mem0, A_Wq, A_Wk, A_Wv, A_Wo, A_seg_len, B_x, B_w_r, B_w_gate, B_w_up, B_w_down):
        del B_x
        B, S, D = A_x.shape
        _, H, DH = A_Wq.shape
        M = A_mem0.shape[1]
        F = B_w_gate.shape[1]
        SEG = int(A_seg_len)
        assert B == 1
        NSEG = S // SEG
        any_spec = pl.BlockSpec(memory_space=pl.ANY)
        out = pl.pallas_call(
            _make_kernel(S, D, H, DH, M, SEG, F, cfg),
            out_shape=jax.ShapeDtypeStruct((S, D), A_x.dtype),
            in_specs=[any_spec] * 11,
            out_specs=any_spec,
            scratch_shapes=[
                pltpu.VMEM((M, D), BF16),
                pltpu.VMEM((D,), BF16),
                pltpu.VMEM((NSEG, PRE, D), BF16),
                pltpu.VMEM((S, D), BF16),
                pltpu.VMEM(((NSEG + GROUP) * PRE // 2 + NSEG * (SEG - PRE), D), U32),
                pltpu.VMEM((S, D), F32),
                pltpu.VMEM((H // 2, 3, D, DH), U32),
                pltpu.VMEM((H, D // 2, 3 * DH), U32),
                pltpu.VMEM((H * DH // 2, D), U32),
                pltpu.VMEM((H, (NSEG + GROUP) * PRE, 3 * DH), F32),
                pltpu.VMEM((M + SEG, H * DH), F32),
                pltpu.VMEM((SEG, D), F32),
                pltpu.VMEM((F, D), BF16),
                pltpu.VMEM((F, D), BF16),
                pltpu.VMEM((F, D), BF16),
                pltpu.VMEM((2 * TOPK, D), F32),
                pltpu.VMEM((S, D), A_x.dtype),
                pltpu.SMEM((2 * TOPK,), I32),
                pltpu.SemaphoreType.DMA((8,)),
                pltpu.SemaphoreType.DMA((3,)),
                pltpu.SemaphoreType.DMA((3 * H // 2,)),
                pltpu.SemaphoreType.DMA((4,)),
                pltpu.SemaphoreType.DMA((6,)),
                pltpu.SemaphoreType.DMA,
            ],
            compiler_params=pltpu.CompilerParams(
                vmem_limit_bytes=120 * 2**20,
                disable_bounds_checks=cfg.get("nobc", False), flags=cfg.get("flags")),
        )(A_x.reshape(S, D), A_x.reshape(NSEG, SEG // PRE, PRE, D), A_mem0.reshape(M, D),
          A_Wq, A_Wk, A_Wv, A_Wo.reshape(H * DH, D),
          B_w_r, B_w_gate.T, B_w_up.T, B_w_down)
        return out.reshape(B, S, D)

    return fn


pallas_recurrent_scan__memory_aug_recurrent_mem_tr__moe_arch_mod__prompt_kernel = build({})
```

```python
import functools

import jax
import jax.numpy as jnp
from jax import lax
from jax.experimental import pallas as pl
from jax.experimental.pallas import tpu as pltpu

F32 = jnp.float32
BF16 = jnp.bfloat16
U32 = jnp.uint32
I32 = jnp.int32

TOPK = 8
PRE = 8
GROUP = 4
LN_EPS = 1e-05


def _bf(x):
    return x.astype(BF16).astype(F32)


def _layernorm(x):
    d = x.shape[-1]
    mean = jnp.sum(x, axis=-1, keepdims=True) * (1.0 / d)
    xc = x - mean
    var = jnp.sum(xc * xc, axis=-1, keepdims=True) * (1.0 / d)
    den = _bf(jnp.sqrt(_bf(_bf(var) + _bf(jnp.float32(LN_EPS)))))
    return _bf(_bf(x - _bf(mean)) / den)


def _make_kernel(S, D, H, DH, M, SEG, F, cfg):
    NSEG = S // SEG
    L = M + SEG
    MAIN = SEG - PRE
    NPAIR = H // 2
    NGROUP = NSEG // GROUP
    NFULL = NPAIR - GROUP // 2
    LAG_QK, LAG_PV = cfg.get("lag", (2, 2))
    EARLY = cfg.get("early", 1)
    RATE = cfg.get("rate", 4)
    LN_ITERS = 8
    TOPK_ITERS = 3
    LN_ROWS = S // LN_ITERS
    AHEAD = cfg.get("ahead", 3)
    XN0 = (NSEG + GROUP) * PRE // 2
    scale = DH ** -0.5
    nt_dims = (((1,), (1,)), ((), ()))
    assert NFULL == 1 + LN_ITERS + 1 + TOPK_ITERS + 1

    def kernel(x_hbm, x4_hbm, mem0_hbm, wq_hbm, wk_hbm, wv_hbm, wo_hbm, wr_hbm, wg_hbm, wu_hbm, wd_hbm,
               out_hbm,
               mem0_v, wr_v, xtail_v, x_v, xx_v, z_v, stage, wqkv, wo_v, pre_v, o_v, g_v,
               wg_v, wu_v, wd_v, xsel_v, out_v, sel_s,
               sem_x, sem_s, sem_w, sem_o, sem_b, sem_out):
        import contextlib
        _scopes = contextlib.ExitStack()
        def mark(name):
            if cfg.get("scopes"):
                _scopes.close()
                if name:
                    _scopes.enter_context(jax.named_scope(name))
        mark("a_start")
        cp_tail = pltpu.make_async_copy(x4_hbm.at[:, SEG // PRE - 1], xtail_v, sem_s.at[2])
        cp_tail.start()

        def w_copy(p, j):
            src = (wq_hbm, wk_hbm, wv_hbm)[j].bitcast(U32).at[:, p, :]
            return pltpu.make_async_copy(src, stage.at[p, j], sem_w.at[p * 3 + j])

        def w_start(p):
            for j in range(3):
                w_copy(p, j).start()

        def x_copy(i):
            r0 = pl.multiple_of(i * LN_ROWS, LN_ROWS)
            return pltpu.make_async_copy(x_hbm.at[pl.ds(r0, LN_ROWS), :], x_v.at[pl.ds(r0, LN_ROWS), :],
                                         sem_x.at[i])

        cp_s = [pltpu.make_async_copy(wr_hbm, wr_v, sem_s.at[0]),
                pltpu.make_async_copy(mem0_hbm, mem0_v, sem_s.at[1])]

        def pieces(src, dst, n, sem):
            rows = dst.shape[0] // n
            return [pltpu.make_async_copy(src.at[pl.ds(i * rows, rows), :], dst.at[pl.ds(i * rows, rows), :],
                                          sem.at[i]) for i in range(n)]

        late = (pieces(wg_hbm, wg_v, 2, sem_b.at[pl.ds(0, 2)]) + pieces(wu_hbm, wu_v, 2, sem_b.at[pl.ds(2, 2)])
                + pieces(wd_hbm, wd_v, 2, sem_b.at[pl.ds(4, 2)]) + pieces(wo_hbm.bitcast(U32), wo_v, 4, sem_o))

        def w_wait(p):
            for j in range(3):
                w_copy(p, j).wait()

        def unpack(p, j, t=0, n=1):
            rows = D // 2 // n
            a = stage[p, j, pl.ds(2 * t * rows, rows, stride=2), :]
            b = stage[p, j, pl.ds(2 * t * rows + 1, rows, stride=2), :]
            dst = (slice(t * rows, (t + 1) * rows), slice(j * DH, (j + 1) * DH))
            wqkv[(2 * p,) + dst] = (a & 0xFFFF) | (b << 16)
            wqkv[(2 * p + 1,) + dst] = (a >> 16) | (b & jnp.uint32(0xFFFF0000))

        def unpack_jobs(p, n=1):
            return [functools.partial(unpack, p, j, t, n) for j in range(3) for t in range(n)]

        def mix(*lists):
            tagged = [((i + 0.5) / len(l), k, job) for k, l in enumerate(lists) for i, job in enumerate(l)]
            return [job for _, _, job in sorted(tagged, key=lambda e: e[:2])]

        def project(h, r0, rows, j=None):
            cols = slice(None) if j is None else slice(j * DH, (j + 1) * DH)
            lhs = pltpu.bitcast(xx_v[pl.ds(r0 // 2, rows // 2), :], BF16)
            w = pltpu.bitcast(wqkv[h, :, cols], BF16)
            pre_v[h, pl.ds(r0, rows), cols] = jnp.dot(lhs, w, preferred_element_type=F32)

        NCHUNK = cfg.get("nchunk", 8)
        CHUNK = NSEG * PRE // NCHUNK

        def project_pair(p, jobs, fine=False, free=2):
            parts = [(c, j) for c in range(2 * NCHUNK) for j in (range(3) if fine else (None,))]
            m = len(parts) - free
            for i, (c, j) in enumerate(parts):
                project(2 * p + c // NCHUNK, (c % NCHUNK) * CHUNK, CHUNK, j)
                if i < m:
                    for job in jobs[i * len(jobs) // m:(i + 1) * len(jobs) // m]:
                        job()

        ngroup = cfg.get('steps', NGROUP)

        def scan():
            mark('m_wait_wo')
            if not cfg.get('scan_only'):
                for c in late[6:]:
                    c.wait()
            mark('n_scan')
            row = lax.broadcasted_iota(I32, (L, L), 0)
            col = lax.broadcasted_iota(I32, (L, L), 1)
            mask = (row < M) | (row >= col)

            def out_copy(c):
                r0 = pl.multiple_of(c * (GROUP * SEG), GROUP * SEG)
                return pltpu.make_async_copy(out_v.at[pl.ds(r0, GROUP * SEG), :],
                                             out_hbm.at[pl.ds(r0, GROUP * SEG), :], sem_out)

            def step(grp, sub_step, mem):
                s = grp * GROUP + sub_step
                r0 = pl.multiple_of(s * SEG, SEG)
                p0 = pl.multiple_of(s * PRE, PRE)
                xm = pltpu.bitcast(xx_v[pl.ds(pl.multiple_of(XN0 + s * MAIN, 8), MAIN), :], F32)
                hh = jnp.concatenate([mem, xm], axis=0).astype(BF16)
                q, k, v, e, inv = {}, {}, {}, {}, {}
                acc = [None]

                def proj(h, j=None):
                    cols = slice(None) if j is None else slice(j * DH, (j + 1) * DH)
                    t = jnp.dot(hh, pltpu.bitcast(wqkv[h, :, cols], BF16), preferred_element_type=F32)
                    t = jnp.concatenate([t, pre_v[h, pl.ds(p0, PRE), cols]], axis=0)
                    if j is None:
                        q[h] = t[:, 0:DH]
                        k[h] = t[:, DH:2 * DH].astype(BF16)
                        v[h] = t[:, 2 * DH:3 * DH].astype(BF16)
                    else:
                        (q, k, v)[j][h] = t.astype(BF16) if j else t

                def scores(h):
                    sc = lax.dot_general(q.pop(h), k.pop(h), nt_dims, preferred_element_type=F32)
                    sc = jnp.where(mask, sc * scale, -1e9)
                    ex = jnp.exp(sc - jnp.max(sc, axis=-1, keepdims=True))
                    e[h] = ex
                    inv[h] = 1.0 / jnp.sum(ex, axis=-1, keepdims=True)

                def values(h):
                    o = jnp.dot(e.pop(h), v.pop(h), preferred_element_type=F32)
                    o_v[:, h * DH:(h + 1) * DH] = o * inv.pop(h)

                def outproj(h, n):
                    w = pltpu.bitcast(wo_v[h * (DH // 2):(h + n) * (DH // 2), :], BF16)
                    t = jnp.dot(o_v[:, h * DH:(h + n) * DH], w, preferred_element_type=F32)
                    acc[0] = t if acc[0] is None else acc[0] + t

                done = 0
                t = 0
                GO = cfg.get("go", 2)
                while done < H:
                    for what in cfg.get("order", "1s0v2o"):
                        if what == "p" and t < H:
                            proj(t)
                        if what in "012" and t < H:
                            proj(t, int(what))
                        if what == "s" and 0 <= t - LAG_QK < H:
                            scores(t - LAG_QK)
                        if what == "v" and 0 <= t - LAG_QK - LAG_PV < H:
                            values(t - LAG_QK - LAG_PV)
                        if what == "o" and t >= H - EARLY:
                            n = 0
                            while done < H and n < RATE and done + GO - 1 + LAG_QK + LAG_PV + 1 <= t:
                                outproj(done, GO)
                                done += GO
                                n += GO
                    if t == cfg.get("g_at", 8) and not cfg.get("g_first"):
                        z = z_v[pl.ds(r0, SEG), :]
                        g_v[...] = z * jax.nn.sigmoid(z)
                    t += 1

                hf = H - GROUP + sub_step
                f0 = pl.multiple_of((grp + 1) * (GROUP * PRE), GROUP * PRE)
                f1 = pl.multiple_of((grp + 1) * (GROUP * PRE // 2), GROUP * PRE // 2)
                pre_v[hf, pl.ds(f0, GROUP * PRE), :] = jnp.dot(
                    pltpu.bitcast(xx_v[pl.ds(f1, GROUP * PRE // 2), :], BF16),
                    pltpu.bitcast(wqkv[hf], BF16), preferred_element_type=F32)

                res = acc[0]
                x = x_v[pl.ds(r0, SEG), :].astype(F32)
                out_v[pl.ds(r0, SEG), :] = (x + res[M:] * g_v[...]).astype(out_v.dtype)
                return res[:M]

            UG = cfg.get("ug", 1)

            def group_body(i, mem):
                for g in range(UG):
                    for k in range(GROUP):
                        mem = step(i * UG + g, k, mem)
                if cfg.get("oc"):
                    cuts = cfg["oc"]
                    for lo, hi in zip(cuts[:-1], cuts[1:]):
                        @pl.when(i == hi - 1)
                        def _():
                            rows = pl.ds(lo * GROUP * SEG, (hi - lo) * GROUP * SEG)
                            pltpu.make_async_copy(out_v.at[rows, :], out_hbm.at[rows, :], sem_out).start()
                else:
                    for g in range(UG):
                        out_copy(i * UG + g).start()
                return mem

            lax.fori_loop(0, ngroup // UG, group_body, mem0_v[...].astype(F32))
        def scan_only():
            cp_tail.wait()
            scan()
            pltpu.make_async_copy(out_v, out_hbm, sem_out).wait()

        def ln_tail(i, n):
            xn = _layernorm(xtail_v[i * n:(i + 1) * n].astype(F32).reshape(n * PRE, D))
            xx_v[i * n * PRE // 2:(i + 1) * n * PRE // 2, :] = pltpu.bitcast(xn.astype(BF16), U32)
            for k in range(n):
                z_v[pl.ds((i * n + k) * SEG + MAIN, PRE), :] = xn[k * PRE:(k + 1) * PRE]

        if cfg.get('scan_only'):
            return scan_only()
        mark('b_wait_tail')
        w_start(0)
        cp_tail.wait()
        w_wait(0)
        mark('e_p0')
        w_start(1)
        x_copy(0).start()
        w_start(2)
        NQ = cfg.get("nq", 4)
        ln_tail(0, NSEG // NQ)
        for job in unpack_jobs(0):
            job()
        for i in range(NQ):
            project(0, i * (NSEG * PRE // NQ), NSEG * PRE // NQ)
            if i + 1 < NQ:
                ln_tail(i + 1, NSEG // NQ)
            project(1, i * (NSEG * PRE // NQ), NSEG * PRE // NQ)
        xx_v[NSEG * PRE // 2:XN0, :] = jnp.zeros((GROUP * PRE // 2, D), U32)
        mark('f_unpack1')
        w_wait(1)
        w_start(3)
        x_copy(1).start()
        for c in cp_s:
            c.start()
        for job in unpack_jobs(1):
            job()

        mark('g_ln_loop')

        def ln_body(i, c):
            p = i + 1
            w_wait(p + 1)
            x_copy(i).wait()

            @pl.when(i + 2 < LN_ITERS)
            def _():
                x_copy(i + 2).start()

            w_start(i + 4)
            for at, cp in enumerate(late[:6]):
                @pl.when(i == at + 2)
                def _():
                    cp.start()

            def ln(t):
                seg = i * (LN_ROWS // SEG) + t
                r0 = pl.multiple_of(seg * SEG, SEG)
                xn = _layernorm(x_v[pl.ds(r0, SEG), :].astype(F32)[:MAIN])
                xx_v[pl.ds(pl.multiple_of(XN0 + seg * MAIN, 8), MAIN), :] = pltpu.bitcast(xn, U32)
                z_v[pl.ds(r0, MAIN), :] = xn

            lns = [functools.partial(ln, t) for t in range(LN_ROWS // SEG)]
            u = unpack_jobs(jnp.minimum(p + 1, NPAIR - 1), cfg.get("un", 10))
            project_pair(p, mix(lns, u), free=cfg.get("free", 3))
            return c

        lax.fori_loop(0, LN_ITERS, ln_body, 0)

        mark('h_router')
        p_r = 1 + LN_ITERS
        w_wait(p_r + 1)
        for c in cp_s:
            c.wait()
        w_start(LN_ITERS + 4)
        w_start(LN_ITERS + 5)
        sub = lax.broadcasted_iota(I32, (8, 128), 0)
        wr = jnp.broadcast_to(wr_v[...].astype(F32).reshape(1, D), (8, D))
        parts = [jnp.zeros((8, 128), F32) for _ in range(S // 1024)]

        def score(t):
            xt = z_v[t * 128:(t + 1) * 128, :].astype(BF16)
            r = lax.dot_general(wr, xt, nt_dims, preferred_element_type=F32)
            parts[t // 8] = jnp.where(sub == t % 8, r, parts[t // 8])

        project_pair(p_r, [functools.partial(score, t) for t in range(S // 128)] + unpack_jobs(p_r + 1),
                     fine=True, free=cfg.get("free_r", 16))
        r = _bf(jnp.concatenate(parts, axis=0))
        bits = (pltpu.bitcast(r, U32) >> 16).astype(I32)
        key = jnp.where(bits >= 0x8000, 0xFFFF - bits, bits + 0x8000)
        key = jnp.where(r == 0.0, 0x8000, key)
        key = jnp.where(r != r, -1, key).astype(F32)
        pos = (lax.broadcasted_iota(I32, r.shape, 0) * 128
               + lax.broadcasted_iota(I32, r.shape, 1)).astype(F32)

        mark('i_topk_loop')
        PICKS = -(-TOPK // TOPK_ITERS)

        def all_reduce(op, t):
            return op(op(t, axis=1, keepdims=True), axis=0, keepdims=True)

        def topk_body(i, carry):
            st = {"key": carry[0], "rsel": carry[1]}
            p = p_r + 1 + i
            w_wait(p + 1)

            @pl.when(i == 0)
            def _():
                w_start(LN_ITERS + 6)
                w_start(LN_ITERS + 7)

            for at in range(2):
                @pl.when(i == at + 1)
                def _():
                    late[6 + 2 * at].start()
                    late[7 + 2 * at].start()

            def best():
                st["best"] = all_reduce(jnp.max, st["key"])

            def first():
                st["where"] = all_reduce(jnp.min, jnp.where(st["key"] == st["best"], pos, float(S)))

            def take(j):
                hit = pos == st["where"]
                st["rsel"] = jnp.where(sub == j, all_reduce(jnp.sum, jnp.where(hit, r, 0.0)), st["rsel"])
                st["key"] = jnp.where(hit, -2.0, st["key"])
                idx = jnp.clip(st["where"].astype(I32)[0, 0], 0, S - 1)
                sel_s[j] = idx
                xsel_v[pl.ds(j, 1), :] = z_v[pl.ds(idx, 1), :]

            jobs = []
            u = unpack_jobs(jnp.minimum(p + 1, NPAIR - 1) if cfg.get("pin_k", True) else p + 1, cfg.get("un", 10))
            for t in range(PICKS):
                jobs += [best, first, functools.partial(take, i * PICKS + t)]
            project_pair(p, mix(jobs, u), free=cfg.get("free_k", 2))
            return st["key"], st["rsel"]

        _, rsel = lax.fori_loop(0, TOPK_ITERS, topk_body, (key, jnp.zeros((8, 128), F32)))

        mark('k_wait_b')
        for c in late[:6]:
            c.wait()
        for p in range(NFULL, NPAIR):
            w_wait(p)
        mark('l_mlp')
        xs = xsel_v[0:TOPK, :]
        mlp = {}

        def hidden(name, ref, t):
            w = ref[t * 128:min((t + 1) * 128, F), :]
            mlp[name, t] = lax.dot_general(xs, w, nt_dims, preferred_element_type=F32)

        def down(t):
            gate = mlp.pop(("g", t))
            act = gate * jax.nn.sigmoid(gate) * mlp.pop(("u", t))
            y = jnp.dot(act, wd_v[t * 128:min((t + 1) * 128, F), :], preferred_element_type=F32)
            mlp["y"] = y + mlp["y"] if "y" in mlp else y

        jobs = []
        NF = -(-F // 128)
        for t in range(NF + 1):
            if t < NF:
                jobs += [functools.partial(hidden, "g", wg_v, t), functools.partial(hidden, "u", wu_v, t)]
            if t > 0:
                jobs += [functools.partial(down, t - 1)]
        for p in range(NFULL, NPAIR):
            for k, job in enumerate(unpack_jobs(p)):
                jobs.insert(4 * k + 2, job)
        project_pair(NFULL - 1, jobs, fine=True, free=cfg.get("free_m", 0))
        for h in range(2 * NFULL, H):
            project(h, 0, GROUP * PRE)
        zsel = xs + mlp["y"] * jax.nn.sigmoid(rsel[:, 0:1])
        for j in range(TOPK):
            z_v[pl.ds(sel_s[j], 1), :] = zsel[j:j + 1, :]

        scan()
        mark('o_out')
        if ngroup == NGROUP:
            pltpu.make_async_copy(out_v, out_hbm, sem_out).wait()
        else:
            for c in range(ngroup):
                out_copy(c).wait()
        mark(None)

    return kernel


def build(cfg):
    @functools.partial(jax.jit, static_argnames=("A_seg_len",))
    def fn(A_x, A_mem0, A_Wq, A_Wk, A_Wv, A_Wo, A_seg_len, B_x, B_w_r, B_w_gate, B_w_up, B_w_down):
        del B_x
        B, S, D = A_x.shape
        _, H, DH = A_Wq.shape
        M = A_mem0.shape[1]
        F = B_w_gate.shape[1]
        SEG = int(A_seg_len)
        assert B == 1
        NSEG = S // SEG
        any_spec = pl.BlockSpec(memory_space=pl.ANY)
        out = pl.pallas_call(
            _make_kernel(S, D, H, DH, M, SEG, F, cfg),
            out_shape=jax.ShapeDtypeStruct((S, D), A_x.dtype),
            in_specs=[any_spec] * 11,
            out_specs=any_spec,
            scratch_shapes=[
                pltpu.VMEM((M, D), BF16),
                pltpu.VMEM((D,), BF16),
                pltpu.VMEM((NSEG, PRE, D), BF16),
                pltpu.VMEM((S, D), BF16),
                pltpu.VMEM(((NSEG + GROUP) * PRE // 2 + NSEG * (SEG - PRE), D), U32),
                pltpu.VMEM((S, D), F32),
                pltpu.VMEM((H // 2, 3, D, DH), U32),
                pltpu.VMEM((H, D // 2, 3 * DH), U32),
                pltpu.VMEM((H * DH // 2, D), U32),
                pltpu.VMEM((H, (NSEG + GROUP) * PRE, 3 * DH), F32),
                pltpu.VMEM((M + SEG, H * DH), F32),
                pltpu.VMEM((SEG, D), F32),
                pltpu.VMEM((F, D), BF16),
                pltpu.VMEM((F, D), BF16),
                pltpu.VMEM((F, D), BF16),
                pltpu.VMEM((2 * TOPK, D), F32),
                pltpu.VMEM((S, D), A_x.dtype),
                pltpu.SMEM((2 * TOPK,), I32),
                pltpu.SemaphoreType.DMA((8,)),
                pltpu.SemaphoreType.DMA((3,)),
                pltpu.SemaphoreType.DMA((3 * H // 2,)),
                pltpu.SemaphoreType.DMA((4,)),
                pltpu.SemaphoreType.DMA((6,)),
                pltpu.SemaphoreType.DMA,
            ],
            compiler_params=pltpu.CompilerParams(
                vmem_limit_bytes=120 * 2**20,
                disable_bounds_checks=cfg.get("nobc", False), flags=cfg.get("flags")),
        )(A_x.reshape(S, D), A_x.reshape(NSEG, SEG // PRE, PRE, D), A_mem0.reshape(M, D),
          A_Wq, A_Wk, A_Wv, A_Wo.reshape(H * DH, D),
          B_w_r, B_w_gate.T, B_w_up.T, B_w_down)
        return out.reshape(B, S, D)

    return fn


pallas_recurrent_scan__memory_aug_recurrent_mem_tr__moe_arch_mod__prompt_kernel = build({})
```

```python
import functools

import jax
import jax.numpy as jnp
import numpy as np
from jax import lax
from jax.experimental import pallas as pl
from jax.experimental.pallas import tpu as pltpu

F32 = jnp.float32
BF16 = jnp.bfloat16
U32 = jnp.uint32
I32 = jnp.int32

TOPK = 8
PRE = 8
GROUP = 4
LN_ITERS = 8
NT_DIMS = (((1,), (1,)), ((), ()))
LN_EPS = float(np.float32(1e-05).astype(jnp.bfloat16))
HI16 = np.uint32(0xFFFF0000)


def _bf(x):
    return x.astype(BF16).astype(F32)


def _layernorm(x):
    d = x.shape[-1]
    mean = jnp.sum(x, axis=-1, keepdims=True) * (1.0 / d)
    xc = x - mean
    var = jnp.sum(xc * xc, axis=-1, keepdims=True) * (1.0 / d)
    den = _bf(jnp.sqrt(_bf(_bf(var) + LN_EPS)))
    return _bf(_bf(x - _bf(mean)) / den)


def _dot(a, b):
    return jnp.dot(a, b, preferred_element_type=F32)


def _dot_nt(a, b):
    return lax.dot_general(a, b, NT_DIMS, preferred_element_type=F32)


def _bf16_rows(words):
    return pltpu.bitcast(words, BF16)


def _all_reduce(op, t):
    return op(op(t, axis=1, keepdims=True), axis=0, keepdims=True)


def _mix(*lists):
    tagged = [((i + 0.5) / len(jobs), k, job)
              for k, jobs in enumerate(lists) for i, job in enumerate(jobs)]
    return [job for _, _, job in sorted(tagged, key=lambda e: e[:2])]


def _make_kernel(S, D, H, DH, M, SEG, F):
    NSEG = S // SEG
    L = M + SEG
    MAIN = SEG - PRE
    NPAIR = H // 2
    NGROUP = NSEG // GROUP
    NFULL = NPAIR - GROUP // 2
    NAHEAD = NSEG * PRE
    LN_ROWS = S // LN_ITERS
    XN0 = (NAHEAD + GROUP * PRE) // 2
    NCHUNK = 8
    scale = DH ** -0.5
    assert M == 8 and DH == 128 and MAIN % 8 == 0 and (M + MAIN) % 16 == 0
    assert S % 1024 == 0 and NSEG % (GROUP * LN_ITERS) == 0 and NPAIR == 16

    def kernel(x_hbm, x4_hbm, mem0_hbm, wq_hbm, wk_hbm, wv_hbm, wo_hbm, wr_hbm, wg_hbm, wu_hbm, wd_hbm,
               out_hbm,
               mem0_v, wr_v, xtail_v, x_v, xx_v, z_v, stage, wqkv, wo_v, pre_v, o_v, g_v,
               wg_v, wu_v, wd_v, xsel_v, out_v, sel_s,
               sem_x, sem_s, sem_w, sem_wo, sem_b, sem_out):
        cp_tail = pltpu.make_async_copy(x4_hbm.at[:, SEG // PRE - 1], xtail_v, sem_s.at[0])
        cp_small = [pltpu.make_async_copy(wr_hbm, wr_v, sem_s.at[1]),
                    pltpu.make_async_copy(mem0_hbm, mem0_v, sem_s.at[2])]

        def x_copy(i):
            rows = pl.ds(pl.multiple_of(i * LN_ROWS, LN_ROWS), LN_ROWS)
            return pltpu.make_async_copy(x_hbm.at[rows, :], x_v.at[rows, :], sem_x.at[i])

        def w_copy(p, j):
            src = (wq_hbm, wk_hbm, wv_hbm)[j].bitcast(U32).at[:, p, :]
            return pltpu.make_async_copy(src, stage.at[p, j], sem_w.at[p * 3 + j])

        def w_start(p):
            for j in range(3):
                w_copy(p, j).start()

        def w_wait(p):
            for j in range(3):
                w_copy(p, j).wait()

        def pieces(src, dst, n, sem, first):
            rows = dst.shape[0] // n
            return [pltpu.make_async_copy(src.at[pl.ds(i * rows, rows), :], dst.at[pl.ds(i * rows, rows), :],
                                          sem.at[first + i]) for i in range(n)]

        cp_mlp = (pieces(wg_hbm, wg_v, 2, sem_b, 0) + pieces(wu_hbm, wu_v, 2, sem_b, 2)
                  + pieces(wd_hbm, wd_v, 2, sem_b, 4))
        cp_wo = pieces(wo_hbm.bitcast(U32), wo_v, 4, sem_wo, 0)

        def unpack(p, j, t, n):
            rows = D // 2 // n
            a = stage[p, j, pl.ds(2 * t * rows, rows, stride=2), :]
            b = stage[p, j, pl.ds(2 * t * rows + 1, rows, stride=2), :]
            dst = (slice(t * rows, (t + 1) * rows), slice(j * DH, (j + 1) * DH))
            wqkv[(2 * p,) + dst] = (a & 0xFFFF) | (b << 16)
            wqkv[(2 * p + 1,) + dst] = (a >> 16) | (b & HI16)

        def unpack_jobs(p, n=1):
            return [functools.partial(unpack, p, j, t, n) for j in range(3) for t in range(n)]

        def project(h, r0, rows, j=None):
            cols = slice(None) if j is None else slice(j * DH, (j + 1) * DH)
            lhs = _bf16_rows(xx_v[pl.ds(r0 // 2, rows // 2), :])
            pre_v[h, pl.ds(r0, rows), cols] = _dot(lhs, _bf16_rows(wqkv[h, :, cols]))

        def project_pair(p, jobs, free, fine=False):
            chunk = NAHEAD // NCHUNK
            parts = [(c, j) for c in range(2 * NCHUNK) for j in (range(3) if fine else (None,))]
            m = len(parts) - free
            for i, (c, j) in enumerate(parts):
                project(2 * p + c // NCHUNK, (c % NCHUNK) * chunk, chunk, j)
                if i < m:
                    for job in jobs[i * len(jobs) // m:(i + 1) * len(jobs) // m]:
                        job()

        def ln_tail(i, n):
            xn = _layernorm(xtail_v[i * n:(i + 1) * n].astype(F32).reshape(n * PRE, D))
            xx_v[i * n * PRE // 2:(i + 1) * n * PRE // 2, :] = pltpu.bitcast(xn.astype(BF16), U32)
            for k in range(n):
                z_v[pl.ds((i * n + k) * SEG + MAIN, PRE), :] = xn[k * PRE:(k + 1) * PRE]

        cp_tail.start()
        w_start(0)
        cp_tail.wait()
        w_wait(0)
        w_start(1)
        x_copy(0).start()
        w_start(2)
        ln_tail(0, NSEG // 4)
        for job in unpack_jobs(0):
            job()
        for i in range(4):
            project(0, i * (NAHEAD // 4), NAHEAD // 4)
            if i < 3:
                ln_tail(i + 1, NSEG // 4)
            project(1, i * (NAHEAD // 4), NAHEAD // 4)
        xx_v[NAHEAD // 2:XN0, :] = jnp.zeros((XN0 - NAHEAD // 2, D), U32)
        w_wait(1)
        w_start(3)
        x_copy(1).start()
        for cp in cp_small:
            cp.start()
        for job in unpack_jobs(1):
            job()

        def ln_body(i, carry):
            p = i + 1
            w_wait(p + 1)
            x_copy(i).wait()

            @pl.when(i + 2 < LN_ITERS)
            def _():
                x_copy(i + 2).start()

            w_start(i + 4)
            for k in range(NPAIR - LN_ITERS - 4):
                @pl.when(i == k + 2)
                def _():
                    w_start(LN_ITERS + 4 + k)

            for k in range(2):
                @pl.when(i == LN_ITERS - 2 + k)
                def _():
                    cp_mlp[k].start()

            def ln(t):
                seg = i * (LN_ROWS // SEG) + t
                r0 = pl.multiple_of(seg * SEG, SEG)
                xn = _layernorm(x_v[pl.ds(r0, SEG), :].astype(F32)[:MAIN])
                xx_v[pl.ds(pl.multiple_of(XN0 + seg * MAIN, 8), MAIN), :] = pltpu.bitcast(xn, U32)
                z_v[pl.ds(r0, MAIN), :] = xn

            lns = [functools.partial(ln, t) for t in range(LN_ROWS // SEG)]
            project_pair(p, _mix(lns, unpack_jobs(jnp.minimum(p + 1, NPAIR - 1), 10)), free=3)
            return carry

        lax.fori_loop(0, LN_ITERS, ln_body, 0)

        p_route = 1 + LN_ITERS
        for p in range(p_route + 1, NFULL):
            w_wait(p)
        for cp in cp_small:
            cp.wait()
        for cp in cp_mlp[2:] + cp_wo:
            cp.start()
        sub = lax.broadcasted_iota(I32, (8, 128), 0)
        pos = (lax.broadcasted_iota(I32, (S // 128, 128), 0) * 128
               + lax.broadcasted_iota(I32, (S // 128, 128), 1)).astype(F32)
        wr = jnp.broadcast_to(wr_v[...].astype(F32).reshape(1, D), (8, D))
        scores_t = [jnp.zeros((8, 128), F32) for _ in range(S // 1024)]
        route = {"r_sel": jnp.zeros((8, 128), F32)}

        def score(t):
            r = _dot_nt(wr, z_v[t * 128:(t + 1) * 128, :].astype(BF16))
            scores_t[t // 8] = jnp.where(sub == t % 8, r, scores_t[t // 8])

        def rank_keys():
            r = _bf(jnp.concatenate(scores_t, axis=0))
            bits = (pltpu.bitcast(r, U32) >> 16).astype(I32)
            key = jnp.where(bits >= 0x8000, 0xFFFF - bits, bits + 0x8000)
            key = jnp.where(r == 0.0, 0x8000, key)
            route["key"] = jnp.where(r != r, -1, key).astype(F32)
            route["r"] = r

        def best():
            route["best"] = _all_reduce(jnp.max, route["key"])

        def first():
            route["at"] = _all_reduce(jnp.min, jnp.where(route["key"] == route["best"], pos, float(S)))

        def take(j):
            hit = pos == route["at"]
            r_j = _all_reduce(jnp.sum, jnp.where(hit, route["r"], 0.0))
            route["r_sel"] = jnp.where(sub == j, r_j, route["r_sel"])
            route["key"] = jnp.where(hit, -2.0, route["key"])
            idx = jnp.clip(route["at"].astype(I32)[0, 0], 0, S - 1)
            sel_s[j] = idx
            xsel_v[j:j + 1, :] = z_v[pl.ds(idx, 1), :]

        project_pair(p_route, [functools.partial(score, t) for t in range(S // 128)] + unpack_jobs(p_route + 1),
                     free=16, fine=True)
        picks = [rank_keys]
        for j in range(TOPK):
            picks += [best, first, functools.partial(take, j)]
        n = NFULL - 1 - (p_route + 1)
        for i in range(n):
            p = p_route + 1 + i
            project_pair(p, _mix(picks[i * len(picks) // n:(i + 1) * len(picks) // n], unpack_jobs(p + 1, 10)),
                         free=2)

        for cp in cp_mlp:
            cp.wait()
        for p in range(NFULL, NPAIR):
            w_wait(p)
        x_sel = xsel_v[...]
        mlp = {}

        def hidden(name, ref, t):
            mlp[name, t] = _dot_nt(x_sel, ref[t * 128:min((t + 1) * 128, F), :])

        def down(t):
            gate = mlp.pop(("gate", t))
            act = gate * jax.nn.sigmoid(gate) * mlp.pop(("up", t))
            y = _dot(act, wd_v[t * 128:min((t + 1) * 128, F), :])
            mlp["y"] = y + mlp["y"] if "y" in mlp else y

        jobs = []
        nf = pl.cdiv(F, 128)
        for t in range(nf + 1):
            if t < nf:
                jobs += [functools.partial(hidden, "gate", wg_v, t), functools.partial(hidden, "up", wu_v, t)]
            if t > 0:
                jobs += [functools.partial(down, t - 1)]
        for p in range(NFULL, NPAIR):
            for k, job in enumerate(unpack_jobs(p)):
                jobs.insert(4 * k + 2, job)
        project_pair(NFULL - 1, jobs, free=0, fine=True)
        for h in range(2 * NFULL, H):
            project(h, 0, GROUP * PRE)
        z_sel = x_sel + mlp["y"] * jax.nn.sigmoid(route["r_sel"][:, 0:1])
        for j in range(TOPK):
            z_v[pl.ds(sel_s[j], 1), :] = z_sel[j:j + 1, :]

        for cp in cp_wo:
            cp.wait()
        row = lax.broadcasted_iota(I32, (L, L), 0)
        col = lax.broadcasted_iota(I32, (L, L), 1)
        mask = (row < M) | (row >= col)

        def step(grp, i, mem):
            s = grp * GROUP + i
            r0 = pl.multiple_of(s * SEG, SEG)
            p0 = pl.multiple_of(s * PRE, PRE)
            xm = pltpu.bitcast(xx_v[pl.ds(pl.multiple_of(XN0 + s * MAIN, 8), MAIN), :], F32)
            hh = jnp.concatenate([mem, xm], axis=0).astype(BF16)
            q, k, v, e, inv = {}, {}, {}, {}, {}
            acc = []

            def proj(h, j):
                cols = slice(j * DH, (j + 1) * DH)
                t = _dot(hh, _bf16_rows(wqkv[h, :, cols]))
                t = jnp.concatenate([t, pre_v[h, pl.ds(p0, PRE), cols]], axis=0)
                (q, k, v)[j][h] = t if j == 0 else t.astype(BF16)

            def scores(h):
                sc = jnp.where(mask, _dot_nt(q.pop(h), k.pop(h)) * scale, -1e9)
                e[h] = jnp.exp(sc - jnp.max(sc, axis=-1, keepdims=True))
                inv[h] = 1.0 / jnp.sum(e[h], axis=-1, keepdims=True)

            def values(h):
                o_v[:, h * DH:(h + 1) * DH] = _dot(e.pop(h), v.pop(h)) * inv.pop(h)

            def outproj(h):
                t = _dot(o_v[:, h * DH:(h + 2) * DH], _bf16_rows(wo_v[h * (DH // 2):(h + 2) * (DH // 2), :]))
                acc[:] = [acc[0] + t if acc else t]

            t = done = 0
            while done < H:
                if t < H:
                    proj(t, 1)
                if 2 <= t < H + 2:
                    scores(t - 2)
                if t < H:
                    proj(t, 0)
                if 4 <= t < H + 4:
                    values(t - 4)
                if t < H:
                    proj(t, 2)
                if t >= H - 1:
                    for _ in range(2):
                        if done < H and done + 6 <= t:
                            outproj(done)
                            done += 2
                if t == 8:
                    z = z_v[pl.ds(r0, SEG), :]
                    g_v[...] = z * jax.nn.sigmoid(z)
                t += 1

            hf = H - GROUP + i
            ahead = GROUP * PRE
            lhs = _bf16_rows(xx_v[pl.ds(pl.multiple_of((grp + 1) * (ahead // 2), ahead // 2), ahead // 2), :])
            pre_v[hf, pl.ds(pl.multiple_of((grp + 1) * ahead, ahead), ahead), :] = _dot(lhs, _bf16_rows(wqkv[hf]))

            res = acc[0]
            x = x_v[pl.ds(r0, SEG), :].astype(F32)
            out_v[pl.ds(r0, SEG), :] = (x + res[M:] * g_v[...]).astype(out_v.dtype)
            return res[:M]

        def group_body(grp, mem):
            for i in range(GROUP):
                mem = step(grp, i, mem)
            rows = pl.ds(pl.multiple_of(grp * (GROUP * SEG), GROUP * SEG), GROUP * SEG)
            pltpu.make_async_copy(out_v.at[rows, :], out_hbm.at[rows, :], sem_out).start()
            return mem

        lax.fori_loop(0, NGROUP, group_body, mem0_v[...].astype(F32))
        pltpu.make_async_copy(out_v, out_hbm, sem_out).wait()

    return kernel


@functools.partial(jax.jit, static_argnames=("A_seg_len",))
def pallas_recurrent_scan__memory_aug_recurrent_mem_tr__moe_arch_mod__prompt_kernel(
    A_x: jax.Array,
    A_mem0: jax.Array,
    A_Wq: jax.Array,
    A_Wk: jax.Array,
    A_Wv: jax.Array,
    A_Wo: jax.Array,
    A_seg_len: int,
    B_x: jax.Array,
    B_w_r: jax.Array,
    B_w_gate: jax.Array,
    B_w_up: jax.Array,
    B_w_down: jax.Array,
):
    del B_x
    B, S, D = A_x.shape
    _, H, DH = A_Wq.shape
    M = A_mem0.shape[1]
    F = B_w_gate.shape[1]
    SEG = int(A_seg_len)
    NSEG = S // SEG
    assert B == 1
    any_spec = pl.BlockSpec(memory_space=pl.ANY)
    out = pl.pallas_call(
        _make_kernel(S, D, H, DH, M, SEG, F),
        out_shape=jax.ShapeDtypeStruct((S, D), A_x.dtype),
        in_specs=[any_spec] * 11,
        out_specs=any_spec,
        scratch_shapes=[
            pltpu.VMEM((M, D), BF16),
            pltpu.VMEM((D,), BF16),
            pltpu.VMEM((NSEG, PRE, D), BF16),
            pltpu.VMEM((S, D), BF16),
            pltpu.VMEM(((NSEG + GROUP) * PRE // 2 + NSEG * (SEG - PRE), D), U32),
            pltpu.VMEM((S, D), F32),
            pltpu.VMEM((H // 2, 3, D, DH), U32),
            pltpu.VMEM((H, D // 2, 3 * DH), U32),
            pltpu.VMEM((H * DH // 2, D), U32),
            pltpu.VMEM((H, (NSEG + GROUP) * PRE, 3 * DH), F32),
            pltpu.VMEM((M + SEG, H * DH), F32),
            pltpu.VMEM((SEG, D), F32),
            pltpu.VMEM((F, D), BF16),
            pltpu.VMEM((F, D), BF16),
            pltpu.VMEM((F, D), BF16),
            pltpu.VMEM((TOPK, D), F32),
            pltpu.VMEM((S, D), A_x.dtype),
            pltpu.SMEM((TOPK,), I32),
            pltpu.SemaphoreType.DMA((LN_ITERS,)),
            pltpu.SemaphoreType.DMA((3,)),
            pltpu.SemaphoreType.DMA((3 * H // 2,)),
            pltpu.SemaphoreType.DMA((4,)),
            pltpu.SemaphoreType.DMA((6,)),
            pltpu.SemaphoreType.DMA,
        ],
        compiler_params=pltpu.CompilerParams(vmem_limit_bytes=120 * 2**20),
    )(A_x.reshape(S, D), A_x.reshape(NSEG, SEG // PRE, PRE, D), A_mem0.reshape(M, D),
      A_Wq, A_Wk, A_Wv, A_Wo.reshape(H * DH, D),
      B_w_r, B_w_gate.T, B_w_up.T, B_w_down)
    return out.reshape(B, S, D)
```

```python
import functools

import jax
import jax.numpy as jnp
import numpy as np
from jax import lax
from jax.experimental import pallas as pl
from jax.experimental.pallas import tpu as pltpu

F32 = jnp.float32
BF16 = jnp.bfloat16
U32 = jnp.uint32
I32 = jnp.int32

TOPK = 8
PRE = 8
GROUP = 4
LN_ITERS = 8
NT_DIMS = (((1,), (1,)), ((), ()))
LN_EPS = float(np.float32(1e-05).astype(jnp.bfloat16))
HI16 = np.uint32(0xFFFF0000)


def _bf(x):
    return x.astype(BF16).astype(F32)


def _layernorm(x):
    d = x.shape[-1]
    mean = jnp.sum(x, axis=-1, keepdims=True) * (1.0 / d)
    xc = x - mean
    var = jnp.sum(xc * xc, axis=-1, keepdims=True) * (1.0 / d)
    den = _bf(jnp.sqrt(_bf(_bf(var) + LN_EPS)))
    return _bf(_bf(x - _bf(mean)) / den)


def _dot(a, b):
    return jnp.dot(a, b, preferred_element_type=F32)


def _dot_nt(a, b):
    return lax.dot_general(a, b, NT_DIMS, preferred_element_type=F32)


def _bf16_rows(words):
    return pltpu.bitcast(words, BF16)


def _all_reduce(op, t):
    return op(op(t, axis=1, keepdims=True), axis=0, keepdims=True)


def _mix(*lists):
    tagged = [((i + 0.5) / len(jobs), k, job)
              for k, jobs in enumerate(lists) for i, job in enumerate(jobs)]
    return [job for _, _, job in sorted(tagged, key=lambda e: e[:2])]


def _make_kernel(S, D, H, DH, M, SEG, F):
    NSEG = S // SEG
    L = M + SEG
    MAIN = SEG - PRE
    NPAIR = H // 2
    NGROUP = NSEG // GROUP
    NFULL = NPAIR - GROUP // 2
    NAHEAD = NSEG * PRE
    LN_ROWS = S // LN_ITERS
    XN0 = (NAHEAD + GROUP * PRE) // 2
    NCHUNK = 8
    scale = DH ** -0.5
    assert M == 8 and DH == 128 and MAIN % 8 == 0 and (M + MAIN) % 16 == 0
    assert S % 1024 == 0 and NSEG % (GROUP * LN_ITERS) == 0 and NPAIR == 16

    def kernel(x_hbm, x4_hbm, mem0_hbm, wq_hbm, wk_hbm, wv_hbm, wo_hbm, wr_hbm, wg_hbm, wu_hbm, wd_hbm,
               out_hbm,
               mem0_v, wr_v, xtail_v, x_v, xx_v, z_v, stage, wqkv, wo_v, pre_v, o_v, g_v,
               wg_v, wu_v, wd_v, xsel_v, out_v, sel_s,
               sem_x, sem_s, sem_w, sem_wo, sem_b, sem_out):
        cp_tail = pltpu.make_async_copy(x4_hbm.at[:, SEG // PRE - 1], xtail_v, sem_s.at[0])
        cp_small = [pltpu.make_async_copy(wr_hbm, wr_v, sem_s.at[1]),
                    pltpu.make_async_copy(mem0_hbm, mem0_v, sem_s.at[2])]

        def x_copy(i):
            rows = pl.ds(pl.multiple_of(i * LN_ROWS, LN_ROWS), LN_ROWS)
            return pltpu.make_async_copy(x_hbm.at[rows, :], x_v.at[rows, :], sem_x.at[i])

        def w_copy(p, j):
            src = (wq_hbm, wk_hbm, wv_hbm)[j].bitcast(U32).at[:, p, :]
            return pltpu.make_async_copy(src, stage.at[p, j], sem_w.at[p * 3 + j])

        def w_start(p):
            for j in range(3):
                w_copy(p, j).start()

        def w_wait(p):
            for j in range(3):
                w_copy(p, j).wait()

        def pieces(src, dst, n, sem, first):
            rows = dst.shape[0] // n
            return [pltpu.make_async_copy(src.at[pl.ds(i * rows, rows), :], dst.at[pl.ds(i * rows, rows), :],
                                          sem.at[first + i]) for i in range(n)]

        cp_mlp = (pieces(wg_hbm, wg_v, 2, sem_b, 0) + pieces(wu_hbm, wu_v, 2, sem_b, 2)
                  + pieces(wd_hbm, wd_v, 2, sem_b, 4))
        cp_wo = pieces(wo_hbm.bitcast(U32), wo_v, 4, sem_wo, 0)

        def unpack(p, j, t, n):
            rows = D // 2 // n
            a = stage[p, j, pl.ds(2 * t * rows, rows, stride=2), :]
            b = stage[p, j, pl.ds(2 * t * rows + 1, rows, stride=2), :]
            dst = (slice(t * rows, (t + 1) * rows), slice(j * DH, (j + 1) * DH))
            wqkv[(2 * p,) + dst] = (a & 0xFFFF) | (b << 16)
            wqkv[(2 * p + 1,) + dst] = (a >> 16) | (b & HI16)

        def unpack_jobs(p, n=1):
            return [functools.partial(unpack, p, j, t, n) for j in range(3) for t in range(n)]

        def project(h, r0, rows, j=None):
            cols = slice(None) if j is None else slice(j * DH, (j + 1) * DH)
            lhs = _bf16_rows(xx_v[pl.ds(r0 // 2, rows // 2), :])
            pre_v[h, pl.ds(r0, rows), cols] = _dot(lhs, _bf16_rows(wqkv[h, :, cols]))

        def project_pair(p, jobs, free, fine=False):
            chunk = NAHEAD // NCHUNK
            parts = [(c, j) for c in range(2 * NCHUNK) for j in (range(3) if fine else (None,))]
            m = len(parts) - free
            for i, (c, j) in enumerate(parts):
                project(2 * p + c // NCHUNK, (c % NCHUNK) * chunk, chunk, j)
                if i < m:
                    for job in jobs[i * len(jobs) // m:(i + 1) * len(jobs) // m]:
                        job()

        def ln_tail(i, n):
            xn = _layernorm(xtail_v[i * n:(i + 1) * n].astype(F32).reshape(n * PRE, D))
            xx_v[i * n * PRE // 2:(i + 1) * n * PRE // 2, :] = pltpu.bitcast(xn.astype(BF16), U32)
            for k in range(n):
                z_v[pl.ds((i * n + k) * SEG + MAIN, PRE), :] = xn[k * PRE:(k + 1) * PRE]

        cp_tail.start()
        w_start(0)
        cp_tail.wait()
        w_wait(0)
        w_start(1)
        x_copy(0).start()
        w_start(2)
        ln_tail(0, NSEG // 4)
        for job in unpack_jobs(0):
            job()
        for i in range(4):
            project(0, i * (NAHEAD // 4), NAHEAD // 4)
            if i < 3:
                ln_tail(i + 1, NSEG // 4)
            project(1, i * (NAHEAD // 4), NAHEAD // 4)
        xx_v[NAHEAD // 2:XN0, :] = jnp.zeros((XN0 - NAHEAD // 2, D), U32)
        w_wait(1)
        w_start(3)
        x_copy(1).start()
        for cp in cp_small:
            cp.start()
        for job in unpack_jobs(1):
            job()

        def ln_body(i, carry):
            p = i + 1
            w_wait(p + 1)
            x_copy(i).wait()

            @pl.when(i + 2 < LN_ITERS)
            def _():
                x_copy(i + 2).start()

            w_start(i + 4)
            for k in range(NPAIR - LN_ITERS - 4):
                @pl.when(i == k + 2)
                def _():
                    w_start(LN_ITERS + 4 + k)

            for k in range(2):
                @pl.when(i == LN_ITERS - 2 + k)
                def _():
                    cp_mlp[k].start()

            normed = {}

            def ln(t):
                r0 = pl.multiple_of((i * (LN_ROWS // SEG) + t) * SEG, SEG)
                normed[t] = _layernorm(x_v[pl.ds(r0, SEG), :].astype(F32)[:MAIN])

            def ln_store(t):
                seg = i * (LN_ROWS // SEG) + t
                xn = normed.pop(t)
                xx_v[pl.ds(pl.multiple_of(XN0 + seg * MAIN, 8), MAIN), :] = pltpu.bitcast(xn, U32)
                z_v[pl.ds(pl.multiple_of(seg * SEG, SEG), MAIN), :] = xn

            jobs = unpack_jobs(jnp.minimum(p + 1, NPAIR - 1), 10)
            for t in range(LN_ROWS // SEG):
                jobs += [functools.partial(ln, t), functools.partial(ln_store, t)]
            project_pair(p, jobs, free=3, fine=True)
            return carry

        lax.fori_loop(0, LN_ITERS, ln_body, 0)

        p_route = 1 + LN_ITERS
        for p in range(p_route + 1, NFULL):
            w_wait(p)
        for cp in cp_small:
            cp.wait()
        for cp in cp_mlp[2:] + cp_wo:
            cp.start()
        sub = lax.broadcasted_iota(I32, (8, 128), 0)
        pos = (lax.broadcasted_iota(I32, (S // 128, 128), 0) * 128
               + lax.broadcasted_iota(I32, (S // 128, 128), 1)).astype(F32)
        wr = jnp.broadcast_to(wr_v[...].astype(F32).reshape(1, D), (8, D))
        scores_t = [jnp.zeros((8, 128), F32) for _ in range(S // 1024)]
        route = {"r_sel": jnp.zeros((8, 128), F32)}

        def score(t):
            r = _dot_nt(wr, z_v[t * 128:(t + 1) * 128, :].astype(BF16))
            scores_t[t // 8] = jnp.where(sub == t % 8, r, scores_t[t // 8])

        def rank_keys():
            r = _bf(jnp.concatenate(scores_t, axis=0))
            bits = (pltpu.bitcast(r, U32) >> 16).astype(I32)
            key = jnp.where(bits >= 0x8000, 0xFFFF - bits, bits + 0x8000)
            key = jnp.where(r == 0.0, 0x8000, key)
            route["key"] = jnp.where(r != r, -1, key).astype(F32)
            route["r"] = r

        def best():
            route["best"] = _all_reduce(jnp.max, route["key"])

        def first():
            route["at"] = _all_reduce(jnp.min, jnp.where(route["key"] == route["best"], pos, float(S)))

        def take(j):
            hit = pos == route["at"]
            r_j = _all_reduce(jnp.sum, jnp.where(hit, route["r"], 0.0))
            route["r_sel"] = jnp.where(sub == j, r_j, route["r_sel"])
            route["key"] = jnp.where(hit, -2.0, route["key"])
            idx = jnp.clip(route["at"].astype(I32)[0, 0], 0, S - 1)
            sel_s[j] = idx
            xsel_v[j:j + 1, :] = z_v[pl.ds(idx, 1), :]

        project_pair(p_route, [functools.partial(score, t) for t in range(S // 128)] + unpack_jobs(p_route + 1),
                     free=8, fine=True)
        picks = [rank_keys]
        for j in range(TOPK):
            picks += [best, first, functools.partial(take, j)]
        n = NFULL - 1 - (p_route + 1)
        for i in range(n):
            p = p_route + 1 + i
            project_pair(p, _mix(picks[i * len(picks) // n:(i + 1) * len(picks) // n], unpack_jobs(p + 1, 10)),
                         free=2)

        for cp in cp_mlp:
            cp.wait()
        for p in range(NFULL, NPAIR):
            w_wait(p)
        x_sel = xsel_v[...]
        mlp = {}

        def hidden(name, ref, t):
            mlp[name, t] = _dot_nt(x_sel, ref[t * 128:min((t + 1) * 128, F), :])

        def down(t):
            gate = mlp.pop(("gate", t))
            act = gate * jax.nn.sigmoid(gate) * mlp.pop(("up", t))
            y = _dot(act, wd_v[t * 128:min((t + 1) * 128, F), :])
            mlp["y"] = y + mlp["y"] if "y" in mlp else y

        jobs = []
        nf = pl.cdiv(F, 128)
        for t in range(nf + 1):
            if t < nf:
                jobs += [functools.partial(hidden, "gate", wg_v, t), functools.partial(hidden, "up", wu_v, t)]
            if t > 0:
                jobs += [functools.partial(down, t - 1)]
        for p in range(NFULL, NPAIR):
            for k, job in enumerate(unpack_jobs(p)):
                jobs.insert(4 * k + 2, job)
        project_pair(NFULL - 1, jobs, free=0, fine=True)
        for h in range(2 * NFULL, H):
            project(h, 0, GROUP * PRE)
        z_sel = x_sel + mlp["y"] * jax.nn.sigmoid(route["r_sel"][:, 0:1])
        for j in range(TOPK):
            z_v[pl.ds(sel_s[j], 1), :] = z_sel[j:j + 1, :]

        for cp in cp_wo:
            cp.wait()
        row = lax.broadcasted_iota(I32, (L, L), 0)
        col = lax.broadcasted_iota(I32, (L, L), 1)
        mask = (row < M) | (row >= col)

        def step(grp, i, mem):
            s = grp * GROUP + i
            r0 = pl.multiple_of(s * SEG, SEG)
            p0 = pl.multiple_of(s * PRE, PRE)
            xm = pltpu.bitcast(xx_v[pl.ds(pl.multiple_of(XN0 + s * MAIN, 8), MAIN), :], F32)
            hh = jnp.concatenate([mem, xm], axis=0).astype(BF16)
            q, k, v, e, inv = {}, {}, {}, {}, {}
            acc = []

            def proj(h, j):
                cols = slice(j * DH, (j + 1) * DH)
                t = _dot(hh, _bf16_rows(wqkv[h, :, cols]))
                t = jnp.concatenate([t, pre_v[h, pl.ds(p0, PRE), cols]], axis=0)
                (q, k, v)[j][h] = t if j == 0 else t.astype(BF16)

            def scores(h):
                sc = jnp.where(mask, _dot_nt(q.pop(h), k.pop(h)) * scale, -1e9)
                e[h] = jnp.exp(sc - jnp.max(sc, axis=-1, keepdims=True))
                inv[h] = 1.0 / jnp.sum(e[h], axis=-1, keepdims=True)

            def values(h):
                o_v[:, h * DH:(h + 1) * DH] = _dot(e.pop(h), v.pop(h)) * inv.pop(h)

            def outproj(h):
                t = _dot(o_v[:, h * DH:(h + 2) * DH], _bf16_rows(wo_v[h * (DH // 2):(h + 2) * (DH // 2), :]))
                acc[:] = [acc[0] + t if acc else t]

            t = done = 0
            while done < H:
                if t < H:
                    proj(t, 1)
                if 2 <= t < H + 2:
                    scores(t - 2)
                if t < H:
                    proj(t, 0)
                if 4 <= t < H + 4:
                    values(t - 4)
                if t < H:
                    proj(t, 2)
                if t >= H - 1:
                    for _ in range(2):
                        if done < H and done + 6 <= t:
                            outproj(done)
                            done += 2
                if t == 8:
                    z = z_v[pl.ds(r0, SEG), :]
                    g_v[...] = z * jax.nn.sigmoid(z)
                t += 1

            hf = H - GROUP + i
            ahead = GROUP * PRE
            lhs = _bf16_rows(xx_v[pl.ds(pl.multiple_of((grp + 1) * (ahead // 2), ahead // 2), ahead // 2), :])
            pre_v[hf, pl.ds(pl.multiple_of((grp + 1) * ahead, ahead), ahead), :] = _dot(lhs, _bf16_rows(wqkv[hf]))

            res = acc[0]
            x = x_v[pl.ds(r0, SEG), :].astype(F32)
            out_v[pl.ds(r0, SEG), :] = (x + res[M:] * g_v[...]).astype(out_v.dtype)
            return res[:M]

        def group_body(grp, mem):
            for i in range(GROUP):
                mem = step(grp, i, mem)
            rows = pl.ds(pl.multiple_of(grp * (GROUP * SEG), GROUP * SEG), GROUP * SEG)
            pltpu.make_async_copy(out_v.at[rows, :], out_hbm.at[rows, :], sem_out).start()
            return mem

        lax.fori_loop(0, NGROUP, group_body, mem0_v[...].astype(F32))
        pltpu.make_async_copy(out_v, out_hbm, sem_out).wait()

    return kernel


@functools.partial(jax.jit, static_argnames=("A_seg_len",))
def pallas_recurrent_scan__memory_aug_recurrent_mem_tr__moe_arch_mod__prompt_kernel(
    A_x: jax.Array,
    A_mem0: jax.Array,
    A_Wq: jax.Array,
    A_Wk: jax.Array,
    A_Wv: jax.Array,
    A_Wo: jax.Array,
    A_seg_len: int,
    B_x: jax.Array,
    B_w_r: jax.Array,
    B_w_gate: jax.Array,
    B_w_up: jax.Array,
    B_w_down: jax.Array,
):
    del B_x
    B, S, D = A_x.shape
    _, H, DH = A_Wq.shape
    M = A_mem0.shape[1]
    F = B_w_gate.shape[1]
    SEG = int(A_seg_len)
    NSEG = S // SEG
    assert B == 1
    any_spec = pl.BlockSpec(memory_space=pl.ANY)
    out = pl.pallas_call(
        _make_kernel(S, D, H, DH, M, SEG, F),
        out_shape=jax.ShapeDtypeStruct((S, D), A_x.dtype),
        in_specs=[any_spec] * 11,
        out_specs=any_spec,
        scratch_shapes=[
            pltpu.VMEM((M, D), BF16),
            pltpu.VMEM((D,), BF16),
            pltpu.VMEM((NSEG, PRE, D), BF16),
            pltpu.VMEM((S, D), BF16),
            pltpu.VMEM(((NSEG + GROUP) * PRE // 2 + NSEG * (SEG - PRE), D), U32),
            pltpu.VMEM((S, D), F32),
            pltpu.VMEM((H // 2, 3, D, DH), U32),
            pltpu.VMEM((H, D // 2, 3 * DH), U32),
            pltpu.VMEM((H * DH // 2, D), U32),
            pltpu.VMEM((H, (NSEG + GROUP) * PRE, 3 * DH), F32),
            pltpu.VMEM((M + SEG, H * DH), F32),
            pltpu.VMEM((SEG, D), F32),
            pltpu.VMEM((F, D), BF16),
            pltpu.VMEM((F, D), BF16),
            pltpu.VMEM((F, D), BF16),
            pltpu.VMEM((TOPK, D), F32),
            pltpu.VMEM((S, D), A_x.dtype),
            pltpu.SMEM((TOPK,), I32),
            pltpu.SemaphoreType.DMA((LN_ITERS,)),
            pltpu.SemaphoreType.DMA((3,)),
            pltpu.SemaphoreType.DMA((3 * H // 2,)),
            pltpu.SemaphoreType.DMA((4,)),
            pltpu.SemaphoreType.DMA((6,)),
            pltpu.SemaphoreType.DMA,
        ],
        compiler_params=pltpu.CompilerParams(vmem_limit_bytes=120 * 2**20),
    )(A_x.reshape(S, D), A_x.reshape(NSEG, SEG // PRE, PRE, D), A_mem0.reshape(M, D),
      A_Wq, A_Wk, A_Wv, A_Wo.reshape(H * DH, D),
      B_w_r, B_w_gate.T, B_w_up.T, B_w_down)
    return out.reshape(B, S, D)
```
